```python
import jax
import jax.numpy as jnp

def _softmax(x, axis=-1):
    return jax.nn.softmax(x, axis=axis)
def _gelu(x):
    return jax.nn.gelu(x, approximate=True)
def _silu(x):
    return jax.nn.silu(x)
def _sigmoid(x):
    return jax.nn.sigmoid(x)
def _layernorm(x, axis=-1, eps=1e-5):
    m = jnp.mean(x, axis=axis, keepdims=True)
    v = jnp.var(x, axis=axis, keepdims=True)
    return (x - m) / jnp.sqrt(v + eps)
def _scatter_add(tgt, idx, src, axis=0):
    return tgt.at[idx].add(src)
def _segment_sum(src, seg, n):
    return jax.ops.segment_sum(src, seg, n)
class _Rng:
    def __init__(self, key):
        self._k = key
    def _next(self):
        self._k, sub = jax.random.split(self._k)
        return sub
    def normal(self, shape):
        return jax.random.normal(self._next(), shape, dtype=jnp.bfloat16)
    def randint(self, lo, hi, shape):
        return jax.random.randint(self._next(), shape, lo, hi, dtype=jnp.int32)
    def uniform(self, shape, lo=0.0, hi=1.0):
        return jax.random.uniform(self._next(), shape, jnp.bfloat16, lo, hi)
    def permutation(self, n):
        return jax.random.permutation(self._next(), n)


kernel_name = 'concat_heads__compressed_kv_cla__spectral_gfnet__prompt'

def setup_inputs():
    _rng = _Rng(jax.random.key(int.from_bytes(__import__("os").urandom(4), "little")))
    _w = (lambda a: (lambda t: t.astype(jnp.bfloat16) if jnp.issubdtype(t.dtype, jnp.floating) else t)(jnp.asarray(a)))
    def _A_setup():
        B, H, Sq, Sk, D, M = 1, 32, 2048, 2048, 128, 1024
        Dc = 4 * D
        return {
            "x": _w((lambda *s: _rng.normal(s) * 0.05)(B, Sq, M)),
            "c_kv": _w((lambda *s: _rng.normal(s) * 0.05)(B, Sk, Dc)),
            "w_q": _w((lambda *s: _rng.normal(s) * 0.05)(M, H, D) * (M ** -0.5)),
            "w_uk": _w((lambda *s: _rng.normal(s) * 0.05)(Dc, H, D) * (Dc ** -0.5)),
            "w_uv": _w((lambda *s: _rng.normal(s) * 0.05)(Dc, H, D) * (Dc ** -0.5)),
            "w_o": _w((lambda *s: _rng.normal(s) * 0.05)(H, D, M) * ((H * D) ** -0.5)),
        }
    _A_in = _A_setup()

    def _B_setup():
        B, S, D = 1, 2048, 1024
        Df = D // 2 + 1
        return {
            "x": _w((lambda *s: _rng.normal(s) * 0.05)(B, S, D)),
            "w_r": _w((lambda *s: _rng.normal(s) * 0.05)(S, Df) * 0.02),
            "w_i": _w((lambda *s: _rng.normal(s) * 0.05)(S, Df) * 0.02),
        }
    _B_in = _B_setup()

    return {
        "A_x": _A_in["x"],
        "A_c_kv": _A_in["c_kv"],
        "A_w_q": _A_in["w_q"],
        "A_w_uk": _A_in["w_uk"],
        "A_w_uv": _A_in["w_uv"],
        "A_w_o": _A_in["w_o"],
        "B_x": _B_in["x"],
        "B_w_r": _B_in["w_r"],
        "B_w_i": _B_in["w_i"],
    }

def reference(A_x, A_c_kv, A_w_q, A_w_uk, A_w_uv, A_w_o, B_x, B_w_r, B_w_i):
    def _A_ref(x, c_kv, w_q, w_uk, w_uv, w_o):
        B, Sq, M = x.shape[0], x.shape[1], x.shape[2]
        Sk = c_kv.shape[1]
        H, D = w_q.shape[1], w_q.shape[2]
        q = jnp.einsum("bqm,mhd->bhqd", x, w_q)
        k = jnp.einsum("bkc,chd->bhkd", c_kv, w_uk)
        v = jnp.einsum("bkc,chd->bhkd", c_kv, w_uv)
        scores = jnp.einsum("bhqd,bhkd->bhqk", q, k) * (D ** -0.5)
        off = Sk - Sq
        qi = jnp.arange(Sq)[:, None]
        kj = jnp.arange(Sk)[None, :]
        cmask = kj <= (qi + off)
        scores = jnp.where(cmask[None, None], scores, -1e9)
        p = _softmax(scores, axis=-1)
        ctx = jnp.einsum("bhqk,bhkd->bhqd", p, v)
        return jnp.einsum("bhqd,hdm->bqm", ctx, w_o)

    def _B_ref(x, w_r, w_i):
        B, S, D = x.shape
        X = (lambda x, axes=(-2,-1): jnp.fft.rfft2(x.astype(jnp.float32), axes=axes))(x, axes=(-2, -1))
        W = w_r + 1j * w_i
        X = X * W
        y = (lambda x, s, axes=(-2,-1): jnp.fft.irfft2(x, s=s, axes=axes).astype(jnp.bfloat16))(X, (S, D), axes=(-2, -1))
        return y

    a = _A_ref(A_x, A_c_kv, A_w_q, A_w_uk, A_w_uv, A_w_o)
    b = _B_ref(B_x, B_w_r, B_w_i)
    return jnp.concatenate([a, b], axis=-1)
```

```python
import math

import jax
import jax.numpy as jnp
import numpy as np
from jax import lax
from jax.experimental import pallas as pl
from jax.experimental.pallas import tpu as pltpu

S = 2048
DM = 1024
DC = 512
H = 32
HD = 128
T = 128
NG = 4
DF = DM // 2 + 1
NCT = 5
N1, N2 = 32, 64

F32, BF16, U32 = jnp.float32, jnp.bfloat16, jnp.uint32
LOG2E = math.log2(math.e)
Q_SCALE = float(HD ** -0.5 * LOG2E)
MASK_VAL = float(-1e9 * LOG2E)
CLASS_PAIRS = ((0, 4), (1, 7), (2, 6), (3, 5))


def _make_constants():
    b = np.arange(128)[:, None].astype(np.float64)
    m = np.arange(64)[None, :].astype(np.float64)

    def cs(r):
        th = 2.0 * np.pi * b * (r + 8.0 * m) / DM
        return np.cos(th), np.sin(th)

    gdf = np.zeros((4, 256, 256))
    c0, s0 = cs(0)
    c4, s4 = cs(4)
    gdf[0, :128, 0:64], gdf[0, :128, 128:192] = c0, -s0
    gdf[0, 128:, 64:128], gdf[0, 128:, 192:256] = c4, -s4
    for p in (1, 2, 3):
        r, r2 = CLASS_PAIRS[p]
        c, s = cs(r)
        c2, s2 = cs(r2)
        gdf[p, :128, 0:64], gdf[p, 128:, 0:64] = c, s
        gdf[p, :128, 64:128], gdf[p, 128:, 64:128] = c2, -s2
        gdf[p, :128, 128:192], gdf[p, 128:, 128:192] = -s, c
        gdf[p, :128, 192:256], gdf[p, 128:, 192:256] = -s2, -c2
    alt = (-1.0) ** np.arange(128)
    gnf = np.zeros((128, 128))
    gnf[:, 0] = alt

    sc = 1.0 / (S * DM)
    gdi = np.zeros((4, 256, 256))
    w0 = np.full((64, 1), 2.0)
    w0[0] = 1.0
    gdi[0, 0:64, 0:128] = (c0.T * w0) * sc
    gdi[0, 128:192, 0:128] = (-s0.T * w0) * sc
    gdi[0, 128, :] = 0.0
    gdi[0, 64:128, 128:256] = 2.0 * c4.T * sc
    gdi[0, 192:256, 128:256] = -2.0 * s4.T * sc
    for p in (1, 2, 3):
        r, r2 = CLASS_PAIRS[p]
        c, s = cs(r)
        c2, s2 = cs(r2)
        f = 2.0 * sc
        gdi[p, 0:64, 0:128], gdi[p, 128:192, 0:128] = f * c.T, -f * s.T
        gdi[p, 64:128, 0:128], gdi[p, 192:256, 0:128] = f * c2.T, -f * s2.T
        gdi[p, 0:64, 128:256], gdi[p, 128:192, 128:256] = f * s.T, f * c.T
        gdi[p, 64:128, 128:256], gdi[p, 192:256, 128:256] = -f * s2.T, -f * c2.T
    gni = np.zeros((128, 128))
    gni[0, :] = alt * sc

    n2 = np.arange(N2)
    perm = np.concatenate([np.concatenate([8 * j + np.arange(8), 64 + 8 * j + np.arange(8)])
                           for j in range(8)])
    gsf = np.zeros((N1, 128, 128))
    gsi = np.zeros((N1, 128, 128))
    for k1 in range(N1):
        k = k1 + N1 * n2
        g = np.exp(-2j * np.pi * np.outer(k, n2) / S)
        ghat = np.block([[g.real, -g.imag], [g.imag, g.real]])
        gsf[k1] = ghat[perm][:, perm]
        gsi[k1] = ghat.T[perm][:, perm]
    bf = lambda a: np.asarray(a, dtype=np.float32).astype(jnp.bfloat16)
    return bf(gdf), bf(gnf), bf(gdi), bf(gni), bf(gsf), bf(gsi)


_CONSTS = _make_constants()


def _dot(a, b):
    return jnp.dot(a, b, preferred_element_type=F32)


def _dot_nt(a, b):
    return lax.dot_general(a, b, (((1,), (1,)), ((), ())), preferred_element_type=F32)


def _cmul_const(x, e, n, sign):
    re, im = x
    e %= n
    if e == 0:
        return re, im
    if 8 * e % n == 0:
        o = 8 * e // n
        if sign < 0:
            o = (8 - o) % 8
        h = math.sqrt(0.5)
        if o == 2:
            return -im, re
        if o == 4:
            return -re, -im
        if o == 6:
            return im, -re
        if o == 1:
            return (re - im) * h, (re + im) * h
        if o == 3:
            return (re + im) * (-h), (re - im) * h
        if o == 5:
            return (im - re) * h, (re + im) * (-h)
        if o == 7:
            return (re + im) * h, (im - re) * h
    th = sign * 2.0 * math.pi * e / n
    c, s = math.cos(th), math.sin(th)
    return re * c - im * s, re * s + im * c


def _cadd(a, b):
    return a[0] + b[0], a[1] + b[1]


def _csub(a, b):
    return a[0] - b[0], a[1] - b[1]


def _fft(xs, sign):
    n = len(xs)
    if n == 1:
        return xs
    if n == 2:
        return [_cadd(xs[0], xs[1]), _csub(xs[0], xs[1])]
    u = _fft(xs[0::2], sign)
    z1 = _fft(xs[1::4], sign)
    z3 = _fft(xs[3::4], sign)
    out = [None] * n
    q = n // 4
    for k in range(q):
        a = _cmul_const(z1[k], k, n, sign)
        b = _cmul_const(z3[k], 3 * k, n, sign)
        sm, df = _cadd(a, b), _csub(a, b)
        out[k] = _cadd(u[k], sm)
        out[k + 2 * q] = _csub(u[k], sm)
        if sign < 0:
            out[k + q] = (u[k + q][0] + df[1], u[k + q][1] - df[0])
            out[k + 3 * q] = (u[k + q][0] - df[1], u[k + q][1] + df[0])
        else:
            out[k + q] = (u[k + q][0] - df[1], u[k + q][1] + df[0])
            out[k + 3 * q] = (u[k + q][0] + df[1], u[k + q][1] - df[0])
    return out


def _b_prepare_w(wrT_s, wiT_s, wd_s, wt_s):
    def words(a, b):
        return (pltpu.bitcast(a.astype(F32), U32) >> 16) | (
            pltpu.bitcast(b.astype(F32), U32) & jnp.uint32(0xFFFF0000))

    def stage_a(t, c):
        cols = pl.ds(pl.multiple_of(t * T, T), T)
        wd_s[t] = words(wrT_s[0:512, cols], wiT_s[0:512, cols])
        return c
    lax.fori_loop(0, S // T, stage_a, 0)

    def stage_b(t, c):
        rows = pl.ds(pl.multiple_of(t * T, T), T)
        for p, (r, r2) in enumerate(CLASS_PAIRS):
            a = wd_s[t, pl.ds(r, 64, stride=8), :]
            b = wd_s[t, pl.ds(r2, 64, stride=8), :]
            wt_s[p, rows, :] = jnp.concatenate([a, b], axis=0).T
        ny = words(wrT_s[512:513, rows], wiT_s[512:513, rows])
        row = lax.broadcasted_iota(jnp.int32, (T, T), 0)
        wt_s[4, rows, :] = jnp.where(row == 0, jnp.broadcast_to(ny, (T, T)), jnp.uint32(0)).T
        return c
    lax.fori_loop(0, S // T, stage_b, 0)


def _b_d_forward(xb_s, gdf_s, gnf_s, xre_s, xim_s, r0, rows):
    sl = pl.ds(r0, rows)
    x = [xb_s[sl, a * T:(a + 1) * T].astype(F32) for a in range(8)]
    s04, t = x[0] + x[4], x[0] - x[4]
    s26, u = x[2] + x[6], x[2] - x[6]
    s15, v = x[1] + x[5], x[1] - x[5]
    s37, w = x[3] + x[7], x[3] - x[7]
    e, f = s04 + s26, s04 - s26
    g, hh = s15 + s37, s15 - s37
    k = math.sqrt(0.5)
    al, be = (v - w) * k, (v + w) * k
    ys = ((e + g, e - g),
          (t + al, -(u + be)),
          (f, -hh),
          (t - al, u - be))
    for p in range(4):
        lhs = jnp.concatenate([ys[p][0], ys[p][1]], axis=1).astype(BF16)
        o = _dot(lhs, gdf_s[p])
        xre_s[p, sl, :] = o[:, :T]
        xim_s[p, sl, :] = o[:, T:]
    xre_s[4, sl, :] = _dot(ys[0][0].astype(BF16), gnf_s[...])
    xim_s[4, sl, :] = jnp.zeros((rows, T), F32)


def _b_s_pass1(xre_s, xim_s, ys_s, c, j):
    off = pl.multiple_of(j * 8, 8)
    xs = [(xre_s[c, pl.ds(N2 * n1 + off, 8), :], xim_s[c, pl.ds(N2 * n1 + off, 8), :])
          for n1 in range(N1)]
    out = _fft(xs, -1)
    o16 = pl.multiple_of(j * 16, 16)
    for k1 in range(N1):
        ys_s[k1, c, pl.ds(o16, 16), :] = jnp.concatenate(out[k1], axis=0).astype(BF16)


def _b_s_pass2(ys_s, zs_s, wt_s, gsf_s, gsi_s, k1):
    rhs = jnp.concatenate([ys_s[k1, c] for c in range(NCT)], axis=1)
    vv = _dot(gsf_s[k1], rhs)
    outs = []
    for c in range(NCT):
        wd = wt_s[c, pl.ds(k1, N2, stride=N1), :]
        wr = pltpu.bitcast(wd << 16, F32)
        wi = pltpu.bitcast(wd & jnp.uint32(0xFFFF0000), F32)
        pcs = []
        for j in range(8):
            vr = vv[16 * j:16 * j + 8, c * T:(c + 1) * T]
            vi = vv[16 * j + 8:16 * j + 16, c * T:(c + 1) * T]
            a, b = wr[8 * j:8 * j + 8], wi[8 * j:8 * j + 8]
            pcs.append(vr * a - vi * b)
            pcs.append(vr * b + vi * a)
        outs.append(jnp.concatenate(pcs, axis=0))
    pp = jnp.concatenate(outs, axis=1).astype(BF16)
    zz = _dot(gsi_s[k1], pp)
    for c in range(NCT):
        zs_s[k1, c] = zz[:, c * T:(c + 1) * T].astype(BF16)


def _b_s_pass3(zs_s, xre_s, xim_s, c, j):
    o16 = pl.multiple_of(j * 16, 16)
    zs = []
    for k1 in range(N1):
        z = zs_s[k1, c, pl.ds(o16, 16), :].astype(F32)
        zs.append((z[0:8], z[8:16]))
    out = _fft(zs, +1)
    off = pl.multiple_of(j * 8, 8)
    for n1 in range(N1):
        xre_s[c, pl.ds(N2 * n1 + off, 8), :] = out[n1][0]
        xim_s[c, pl.ds(N2 * n1 + off, 8), :] = out[n1][1]


def _b_d_inverse(xre_s, xim_s, gdi_s, gni_s, yb_s, r0, rows):
    sl = pl.ds(r0, rows)
    us = []
    for p in range(4):
        lhs = jnp.concatenate([xre_s[p, sl, :], xim_s[p, sl, :]], axis=1).astype(BF16)
        o = _dot(lhs, gdi_s[p])
        us.append((o[:, :T], o[:, T:]))
    u0 = us[0][0] + _dot(xre_s[4, sl, :].astype(BF16), gni_s[...])
    u4 = us[0][1]
    (u1r, u1i), (u2r, u2i), (u3r, u3i) = us[1], us[2], us[3]
    e0, e1 = u0 + u4, u0 - u4
    ev = (e0 + u2r, e1 - u2i, e0 - u2r, e1 + u2i)
    pq, qq = u1r - u3r, u1i + u3i
    k = math.sqrt(0.5)
    od = (u1r + u3r, (pq - qq) * k, u3i - u1i, (pq + qq) * (-k))
    for a in range(4):
        yb_s[sl, a * T:(a + 1) * T] = (ev[a] + od[a]).astype(BF16)
        yb_s[sl, (a + 4) * T:(a + 5) * T] = (ev[a] - od[a]).astype(BF16)


BQ = 256


def _attn_head(q_s, k_s, v_s, h):
    nt = BQ // T
    nblk = S // BQ
    row = lax.broadcasted_iota(jnp.int32, (T, T), 0)
    col = lax.broadcasted_iota(jnp.int32, (T, T), 1)
    causal = col <= row

    def scores(i):
        r0 = i * BQ
        nfull = r0 // T + 1
        tiles = {}
        s = _dot_nt(q_s[h, r0:r0 + BQ, :], k_s[h, 0:nfull * T, :])
        for t in range(nt):
            for j in range(nfull):
                tiles[t, j] = s[t * T:(t + 1) * T, j * T:(j + 1) * T]
        for t in range(1, nt):
            j = nfull - 1 + t
            st = _dot_nt(q_s[h, r0 + t * T:r0 + BQ, :], k_s[h, j * T:(j + 1) * T, :])
            for u in range(t, nt):
                tiles[u, j] = st[(u - t) * T:(u - t + 1) * T]
        for t in range(nt):
            jd = nfull - 1 + t
            tiles[t, jd] = jnp.where(causal, tiles[t, jd], MASK_VAL)
        return tiles

    def softmax_pv(i, tiles):
        r0 = i * BQ
        nfull = r0 // T + 1
        for t in range(nt):
            nk = nfull + t
            mx = tiles[t, 0]
            for j in range(1, nk):
                mx = jnp.maximum(mx, tiles[t, j])
            m = jnp.max(mx, axis=1, keepdims=True)
            lacc = o = None
            for j in range(nk):
                p = jnp.exp2(tiles[t, j] - m)
                lacc = p if lacc is None else lacc + p
                oo = _dot(p.astype(BF16), v_s[h, j * T:(j + 1) * T, :])
                o = oo if o is None else o + oo
            l = jnp.sum(lacc, axis=1, keepdims=True)
            q_s[h, r0 + t * T:r0 + (t + 1) * T, :] = (
                o * pl.reciprocal(l, approx=True)).astype(BF16)

    cur = scores(nblk - 1)
    for i in range(nblk - 1, -1, -1):
        nxt = scores(i - 1) if i > 0 else None
        softmax_pv(i, cur)
        cur = nxt


PR = 512
OR = 512
BR = 256


def _kernel(ax_hbm, ac_hbm, wq_hbm, wuk_hbm, wuv_hbm, wo_hbm, bx_hbm, wrT_hbm, wiT_hbm,
            gdf_hbm, gnf_hbm, gdi_hbm, gni_hbm, gsf_hbm, gsi_hbm,
            out_hbm,
            ax_s, ac_s, wq_s, wuk_s, wuv_s, wo_s, oa_s, sems):
    def copy(src, dst, i):
        return pltpu.make_async_copy(src, dst, sems.at[i])

    def wcopies(g, slot):
        hs = pl.ds(pl.multiple_of(g * 8, 8), 8)
        return (copy(wq_hbm.at[:, hs, :], wq_s.at[slot], 2 + 3 * slot),
                copy(wuk_hbm.at[:, hs, :], wuk_s.at[slot], 3 + 3 * slot),
                copy(wuv_hbm.at[:, hs, :], wuv_s.at[slot], 4 + 3 * slot))

    def b_phase(bx_s, wrT_s, wiT_s, wd_s, wt_s, xre_s, xim_s, ys_s, zs_s,
                gdf_s, gnf_s, gdi_s, gni_s, gsf_s, gsi_s, bsem):
        def bcopy(src, dst, i):
            return pltpu.make_async_copy(src, dst, bsem.at[i])
        nch = S // BR
        xc = [bcopy(bx_hbm.at[pl.ds(i * BR, BR), :], bx_s.at[pl.ds(i * BR, BR), :], i)
              for i in range(nch)]
        cc = [bcopy(gdf_hbm, gdf_s, nch), bcopy(gnf_hbm, gnf_s, nch + 1),
              bcopy(wrT_hbm, wrT_s, nch + 2), bcopy(wiT_hbm, wiT_s, nch + 3),
              bcopy(gsf_hbm, gsf_s, nch + 4), bcopy(gsi_hbm, gsi_s, nch + 5),
              bcopy(gdi_hbm, gdi_s, nch + 6), bcopy(gni_hbm, gni_s, nch + 7)]
        xc[0].start()
        cc[0].start()
        cc[1].start()
        for c in xc[1:]:
            c.start()
        for c in cc[2:]:
            c.start()
        copy(ax_hbm, ax_s, 0).start()
        copy(ac_hbm, ac_s, 1).start()
        for c in wcopies(0, 0):
            c.start()
        copy(wo_hbm, wo_s, 8).start()

        cc[0].wait()
        cc[1].wait()
        for i in range(nch):
            xc[i].wait()
            _b_d_forward(bx_s, gdf_s, gnf_s, xre_s, xim_s, i * BR, BR)
        cc[2].wait()
        cc[3].wait()
        _b_prepare_w(wrT_s, wiT_s, wd_s, wt_s)

        def p1(u, c):
            _b_s_pass1(xre_s, xim_s, ys_s, u // 8, u % 8)
            return c
        lax.fori_loop(0, NCT * 8, p1, 0)
        for c in cc[4:]:
            c.wait()

        def p2(k1, c):
            _b_s_pass2(ys_s, zs_s, wt_s, gsf_s, gsi_s, k1)
            return c
        lax.fori_loop(0, N1, p2, 0)

        def p3(u, c):
            _b_s_pass3(zs_s, xre_s, xim_s, u // 8, u % 8)
            return c
        lax.fori_loop(0, NCT * 8, p3, 0)

        oc = [bcopy(bx_s.at[pl.ds(i * BR, BR), :],
                    out_hbm.at[pl.ds(i * BR, BR), pl.ds(DM, DM)], i) for i in range(nch)]
        for i in range(nch):
            _b_d_inverse(xre_s, xim_s, gdi_s, gni_s, bx_s, i * BR, BR)
            oc[i].start()
        for c in oc:
            c.wait()

    pl.run_scoped(
        b_phase,
        pltpu.VMEM((S, DM), BF16),
        pltpu.VMEM((DF, S), BF16), pltpu.VMEM((DF, S), BF16),
        pltpu.VMEM((S // T, 512, T), U32), pltpu.VMEM((NCT, S, T), U32),
        pltpu.VMEM((NCT, S, T), F32), pltpu.VMEM((NCT, S, T), F32),
        pltpu.VMEM((N1, NCT, T, T), BF16), pltpu.VMEM((N1, NCT, T, T), BF16),
        pltpu.VMEM((4, 256, 256), BF16), pltpu.VMEM((T, T), BF16),
        pltpu.VMEM((4, 256, 256), BF16), pltpu.VMEM((T, T), BF16),
        pltpu.VMEM((N1, T, T), BF16), pltpu.VMEM((N1, T, T), BF16),
        pltpu.SemaphoreType.DMA((S // BR + 8,)),
    )

    def a_phase(q_s, k_s, v_s):
        copy(ax_hbm, ax_s, 0).wait()
        copy(ac_hbm, ac_s, 1).wait()

        def proj_group(g, c):
            slot = g % 2
            for cp in wcopies(g, slot):
                cp.wait()

            @pl.when(g + 1 < NG)
            def _():
                for cp in wcopies(g + 1, 1 - slot):
                    cp.start()

            def chunk(i, cc):
                rows = pl.ds(pl.multiple_of(i * PR, PR), PR)
                q = _dot(ax_s[rows, :], wq_s[slot].reshape(DM, 8 * HD)) * Q_SCALE
                for hh in range(8):
                    q_s[g * 8 + hh, rows, :] = q[:, hh * HD:(hh + 1) * HD].astype(BF16)
                k = _dot(ac_s[rows, :], wuk_s[slot].reshape(DC, 8 * HD))
                for hh in range(8):
                    k_s[g * 8 + hh, rows, :] = k[:, hh * HD:(hh + 1) * HD].astype(BF16)
                v = _dot(ac_s[rows, :], wuv_s[slot].reshape(DC, 8 * HD))
                for hh in range(8):
                    v_s[g * 8 + hh, rows, :] = v[:, hh * HD:(hh + 1) * HD].astype(BF16)
                return cc
            lax.fori_loop(0, S // PR, chunk, 0)
            return c
        lax.fori_loop(0, NG, proj_group, 0)

        def head(h, c):
            _attn_head(q_s, k_s, v_s, h)
            return c
        lax.fori_loop(0, H, head, 0)

        copy(wo_hbm, wo_s, 8).wait()
        nch = S // OR
        oc = [pltpu.make_async_copy(oa_s.at[pl.ds(i * OR, OR), :],
                                    out_hbm.at[pl.ds(i * OR, OR), pl.ds(0, DM)],
                                    sems.at[9 + i]) for i in range(nch)]

        def ochunk(i, c):
            rows = pl.ds(pl.multiple_of(i * OR, OR), OR)
            lhs = jnp.concatenate([q_s[h, rows, :] for h in range(H)], axis=1)
            oa_s[rows, :] = _dot(lhs, wo_s[...]).astype(BF16)
            for ii in range(nch):
                @pl.when(i == ii)
                def _():
                    oc[ii].start()
            return c
        lax.fori_loop(0, nch, ochunk, 0)
        for c in oc:
            c.wait()

    pl.run_scoped(a_phase, *[pltpu.VMEM((H, S, HD), BF16)] * 3)


@jax.jit
def pallas_concat_heads__compressed_kv_cla__spectral_gfnet__prompt_kernel(
    A_x, A_c_kv, A_w_q, A_w_uk, A_w_uv, A_w_o, B_x, B_w_r, B_w_i,
):
    hbm = pl.BlockSpec(memory_space=pl.ANY)
    out = pl.pallas_call(
        _kernel,
        in_specs=[hbm] * 15,
        out_specs=hbm,
        out_shape=jax.ShapeDtypeStruct((S, 2 * DM), BF16),
        scratch_shapes=[
            pltpu.VMEM((S, DM), BF16), pltpu.VMEM((S, DC), BF16),
            pltpu.VMEM((2, DM, 8, HD), BF16), pltpu.VMEM((2, DC, 8, HD), BF16),
            pltpu.VMEM((2, DC, 8, HD), BF16),
            pltpu.VMEM((H * HD, DM), BF16), pltpu.VMEM((S, DM), BF16),
            pltpu.SemaphoreType.DMA((9 + S // OR,)),
        ],
        compiler_params=pltpu.CompilerParams(vmem_limit_bytes=120 * 1024 * 1024),
    )(A_x.reshape(S, DM), A_c_kv.reshape(S, DC), A_w_q, A_w_uk, A_w_uv,
      A_w_o.reshape(H * HD, DM), B_x.reshape(S, DM), B_w_r.T, B_w_i.T, *_CONSTS)
    return out.reshape(1, S, 2 * DM)
```

```python
import functools
import math

import jax
import jax.numpy as jnp
import numpy as np
from jax import lax
from jax.experimental import pallas as pl
from jax.experimental.pallas import tpu as pltpu

S = 2048
DM = 1024
DC = 512
H = 32
HD = 128
T = 128
NG = 4
DF = DM // 2 + 1
NCT = 5
N1, N2 = 32, 64

F32, BF16, U32 = jnp.float32, jnp.bfloat16, jnp.uint32
LOG2E = math.log2(math.e)
Q_SCALE = float(HD ** -0.5 * LOG2E)
MASK_VAL = float(-1e9 * LOG2E)
CLASS_PAIRS = ((0, 4), (1, 7), (2, 6), (3, 5))


def _make_constants():
    b = np.arange(128)[:, None].astype(np.float64)
    m = np.arange(64)[None, :].astype(np.float64)

    def cs(r):
        th = 2.0 * np.pi * b * (r + 8.0 * m) / DM
        return np.cos(th), np.sin(th)

    gdf = np.zeros((4, 256, 256))
    c0, s0 = cs(0)
    c4, s4 = cs(4)
    gdf[0, :128, 0:64], gdf[0, :128, 128:192] = c0, -s0
    gdf[0, 128:, 64:128], gdf[0, 128:, 192:256] = c4, -s4
    for p in (1, 2, 3):
        r, r2 = CLASS_PAIRS[p]
        c, s = cs(r)
        c2, s2 = cs(r2)
        gdf[p, :128, 0:64], gdf[p, 128:, 0:64] = c, s
        gdf[p, :128, 64:128], gdf[p, 128:, 64:128] = c2, -s2
        gdf[p, :128, 128:192], gdf[p, 128:, 128:192] = -s, c
        gdf[p, :128, 192:256], gdf[p, 128:, 192:256] = -s2, -c2
    alt = (-1.0) ** np.arange(128)
    gnf = np.zeros((128, 128))
    gnf[:, 0] = alt

    sc = 1.0 / (S * DM)
    gdi = np.zeros((4, 256, 256))
    w0 = np.full((64, 1), 2.0)
    w0[0] = 1.0
    gdi[0, 0:64, 0:128] = (c0.T * w0) * sc
    gdi[0, 128:192, 0:128] = (-s0.T * w0) * sc
    gdi[0, 128, :] = 0.0
    gdi[0, 64:128, 128:256] = 2.0 * c4.T * sc
    gdi[0, 192:256, 128:256] = -2.0 * s4.T * sc
    for p in (1, 2, 3):
        r, r2 = CLASS_PAIRS[p]
        c, s = cs(r)
        c2, s2 = cs(r2)
        f = 2.0 * sc
        gdi[p, 0:64, 0:128], gdi[p, 128:192, 0:128] = f * c.T, -f * s.T
        gdi[p, 64:128, 0:128], gdi[p, 192:256, 0:128] = f * c2.T, -f * s2.T
        gdi[p, 0:64, 128:256], gdi[p, 128:192, 128:256] = f * s.T, f * c.T
        gdi[p, 64:128, 128:256], gdi[p, 192:256, 128:256] = -f * s2.T, -f * c2.T
    gni = np.zeros((128, 128))
    gni[0, :] = alt * sc

    n2 = np.arange(N2)
    perm = np.concatenate([np.concatenate([8 * j + np.arange(8), 64 + 8 * j + np.arange(8)])
                           for j in range(8)])
    gsf = np.zeros((N1, 128, 128))
    gsi = np.zeros((N1, 128, 128))
    for k1 in range(N1):
        k = k1 + N1 * n2
        g = np.exp(-2j * np.pi * np.outer(k, n2) / S)
        ghat = np.block([[g.real, -g.imag], [g.imag, g.real]])
        gsf[k1] = ghat[perm][:, perm]
        gsi[k1] = ghat.T[perm][:, perm]
    bf = lambda a: np.asarray(a, dtype=np.float32).astype(jnp.bfloat16)
    return bf(gdf), bf(gnf), bf(gdi), bf(gni), bf(gsf), bf(gsi)


_CONSTS = _make_constants()


def _dot(a, b):
    return jnp.dot(a, b, preferred_element_type=F32)


def _dot_nt(a, b):
    return lax.dot_general(a, b, (((1,), (1,)), ((), ())), preferred_element_type=F32)


def _cmul_const(x, e, n, sign):
    re, im = x
    e %= n
    if e == 0:
        return re, im
    if 8 * e % n == 0:
        o = 8 * e // n
        if sign < 0:
            o = (8 - o) % 8
        h = math.sqrt(0.5)
        if o == 2:
            return -im, re
        if o == 4:
            return -re, -im
        if o == 6:
            return im, -re
        if o == 1:
            return (re - im) * h, (re + im) * h
        if o == 3:
            return (re + im) * (-h), (re - im) * h
        if o == 5:
            return (im - re) * h, (re + im) * (-h)
        if o == 7:
            return (re + im) * h, (im - re) * h
    th = sign * 2.0 * math.pi * e / n
    c, s = math.cos(th), math.sin(th)
    return re * c - im * s, re * s + im * c


def _cadd(a, b):
    return a[0] + b[0], a[1] + b[1]


def _csub(a, b):
    return a[0] - b[0], a[1] - b[1]


def _fft(xs, sign):
    n = len(xs)
    if n == 1:
        return xs
    if n == 2:
        return [_cadd(xs[0], xs[1]), _csub(xs[0], xs[1])]
    u = _fft(xs[0::2], sign)
    z1 = _fft(xs[1::4], sign)
    z3 = _fft(xs[3::4], sign)
    out = [None] * n
    q = n // 4
    for k in range(q):
        a = _cmul_const(z1[k], k, n, sign)
        b = _cmul_const(z3[k], 3 * k, n, sign)
        sm, df = _cadd(a, b), _csub(a, b)
        out[k] = _cadd(u[k], sm)
        out[k + 2 * q] = _csub(u[k], sm)
        if sign < 0:
            out[k + q] = (u[k + q][0] + df[1], u[k + q][1] - df[0])
            out[k + 3 * q] = (u[k + q][0] - df[1], u[k + q][1] + df[0])
        else:
            out[k + q] = (u[k + q][0] - df[1], u[k + q][1] + df[0])
            out[k + 3 * q] = (u[k + q][0] + df[1], u[k + q][1] - df[0])
    return out


def _b_prepare_w(wrT_s, wiT_s, wd_s, wt_s, t):
    def words(a, b):
        return (pltpu.bitcast(a.astype(F32), U32) >> 16) | (
            pltpu.bitcast(b.astype(F32), U32) & jnp.uint32(0xFFFF0000))

    rows = pl.ds(pl.multiple_of(t * T, T), T)
    for a in range(0, 512, 64):
        wd_s[t, a:a + 64, :] = words(wrT_s[a:a + 64, rows], wiT_s[a:a + 64, rows])
    for p, (r, r2) in enumerate(CLASS_PAIRS):
        a = wd_s[t, pl.ds(r, 64, stride=8), :]
        b = wd_s[t, pl.ds(r2, 64, stride=8), :]
        wt_s[p, rows, :] = jnp.concatenate([a, b], axis=0).T
    ny = words(wrT_s[512:513, rows], wiT_s[512:513, rows])
    row = lax.broadcasted_iota(jnp.int32, (T, T), 0)
    wt_s[4, rows, :] = jnp.where(row == 0, jnp.broadcast_to(ny, (T, T)), jnp.uint32(0)).T


def _b_d_forward_vpu(xb_s, y_s, slot, r0, rows):
    for a in range(0, rows, VSL):
        _b_d_forward_vpu_slab(xb_s, y_s, slot, r0, a)


def _b_d_forward_vpu_slab(xb_s, y_s, slot, r0, a):
    sl = pl.ds(r0 + a, VSL)
    x = [xb_s[sl, a * T:(a + 1) * T].astype(F32) for a in range(8)]
    s04, t = x[0] + x[4], x[0] - x[4]
    s26, u = x[2] + x[6], x[2] - x[6]
    s15, v = x[1] + x[5], x[1] - x[5]
    s37, w = x[3] + x[7], x[3] - x[7]
    e, f = s04 + s26, s04 - s26
    g, hh = s15 + s37, s15 - s37
    k = math.sqrt(0.5)
    al, be = (v - w) * k, (v + w) * k
    ys = ((e + g, e - g),
          (t + al, -(u + be)),
          (f, -hh),
          (t - al, u - be))
    for p in range(4):
        y_s[slot, a:a + VSL, 2 * p * T:(2 * p + 2) * T] = jnp.concatenate(
            [ys[p][0], ys[p][1]], axis=1).astype(BF16)


def _b_d_forward_mxu(y_s, slot, gdf_s, gnf_s, xre_s, xim_s, r0, a, rows):
    sl = pl.ds(r0 + a, rows)
    for p in range(4):
        o = _dot(y_s[slot, a:a + rows, 2 * p * T:(2 * p + 2) * T], gdf_s[p])
        xre_s[p, sl, :] = o[:, :T]
        xim_s[p, sl, :] = o[:, T:]
    xre_s[4, sl, :] = _dot(y_s[slot, a:a + rows, 0:T], gnf_s[...])
    xim_s[4, sl, :] = jnp.zeros((rows, T), F32)


def _fft32(load, emit, sign):
    half = N1 // 2
    for par in range(2):
        xs = []
        for n in range(half):
            a, b = load(n), load(n + half)
            xs.append(_cadd(a, b) if par == 0 else _cmul_const(_csub(a, b), n, N1, sign))
        out = _fft(xs, sign)
        for q in range(half):
            emit(2 * q + par, out[q])


def _b_s_pass1(xre_s, xim_s, ys_s, c, j):
    off = pl.multiple_of(j * 8, 8)
    o16 = pl.multiple_of(j * 16, 16)

    def load(n1):
        rows = pl.ds(N2 * n1 + off, 8)
        return xre_s[c, rows, :], xim_s[c, rows, :]

    def emit(k1, v):
        ys_s[k1, c, pl.ds(o16, 16), :] = jnp.concatenate(v, axis=0).astype(BF16)
    _fft32(load, emit, -1)


def _b_s_pass2_fwd(ys_s, gsf_s, k1):
    rhs = jnp.concatenate([ys_s[k1, c] for c in range(NCT)], axis=1)
    return _dot(gsf_s[k1], rhs)


def _b_s_pass2_inv(vv, zs_s, wt_s, gsi_s, k1):
    outs = []
    for c in range(NCT):
        wd = wt_s[c, pl.ds(k1, N2, stride=N1), :]
        wr = pltpu.bitcast(wd << 16, F32)
        wi = pltpu.bitcast(wd & jnp.uint32(0xFFFF0000), F32)
        pcs = []
        for j in range(8):
            vr = vv[16 * j:16 * j + 8, c * T:(c + 1) * T]
            vi = vv[16 * j + 8:16 * j + 16, c * T:(c + 1) * T]
            a, b = wr[8 * j:8 * j + 8], wi[8 * j:8 * j + 8]
            pcs.append(vr * a - vi * b)
            pcs.append(vr * b + vi * a)
        outs.append(jnp.concatenate(pcs, axis=0))
    pp = jnp.concatenate(outs, axis=1).astype(BF16)
    zz = _dot(gsi_s[k1], pp)
    for c in range(NCT):
        zs_s[k1, c] = zz[:, c * T:(c + 1) * T].astype(BF16)


def _b_s_pass2(ys_s, zs_s, wt_s, gsf_s, gsi_s, k1s):
    pend = []
    for a in range(len(k1s) + P2D):
        if a < len(k1s):
            pend.append(_b_s_pass2_fwd(ys_s, gsf_s, k1s[a]))
        if a >= P2D:
            _b_s_pass2_inv(pend.pop(0), zs_s, wt_s, gsi_s, k1s[a - P2D])


def _b_s_pass3(zs_s, xre_s, xim_s, c, j, chain):
    o16 = pl.multiple_of(j * 16, 16)
    off = pl.multiple_of(j * 8, 8)

    def load(k1):
        z = zs_s[k1, c, pl.ds(o16, 16), :].astype(F32)
        return z[0:8], z[8:16]

    def emit(n1, v):
        rows = pl.ds(N2 * n1 + off, 8)
        xre_s[c, rows, :] = v[0]
        xim_s[c, rows, :] = v[1]
        if chain and n1 >= N1 - 2:
            zs_s[N1, 0, 0:16, :] = jnp.concatenate(v, axis=0).astype(BF16)
    _fft32(load, emit, +1)


def _b_d_inverse(xre_s, xim_s, gdi_s, gni_s, yb_s, r0, rows):
    sl = pl.ds(r0, rows)
    us = []
    for p in range(4):
        lhs = jnp.concatenate([xre_s[p, sl, :], xim_s[p, sl, :]], axis=1).astype(BF16)
        o = _dot(lhs, gdi_s[p])
        us.append((o[:, :T], o[:, T:]))
    u0 = us[0][0] + _dot(xre_s[4, sl, :].astype(BF16), gni_s[...])
    u4 = us[0][1]
    (u1r, u1i), (u2r, u2i), (u3r, u3i) = us[1], us[2], us[3]
    e0, e1 = u0 + u4, u0 - u4
    ev = (e0 + u2r, e1 - u2i, e0 - u2r, e1 + u2i)
    pq, qq = u1r - u3r, u1i + u3i
    k = math.sqrt(0.5)
    od = (u1r + u3r, (pq - qq) * k, u3i - u1i, (pq + qq) * (-k))
    for a in range(4):
        yb_s[sl, a * T:(a + 1) * T] = (ev[a] + od[a]).astype(BF16)
        yb_s[sl, (a + 4) * T:(a + 5) * T] = (ev[a] - od[a]).astype(BF16)


VSL = 16
BQ = 256
ADEPTH = 1
ACK = 128


def _attn_head(q_s, k_s, v_s, o_s, h, ho):
    nt = BQ // T
    nblk = S // BQ
    row = lax.broadcasted_iota(jnp.int32, (T, T), 0)
    col = lax.broadcasted_iota(jnp.int32, (T, T), 1)
    causal = col <= row

    def scores(i):
        r0 = i * BQ
        nfull = r0 // T + 1
        tiles = {}
        s = _dot_nt(q_s[h, r0:r0 + BQ, :], k_s[h, 0:nfull * T, :])
        for t in range(nt):
            for j in range(nfull):
                tiles[t, j] = s[t * T:(t + 1) * T, j * T:(j + 1) * T]
        for t in range(1, nt):
            j = nfull - 1 + t
            st = _dot_nt(q_s[h, r0 + t * T:r0 + BQ, :], k_s[h, j * T:(j + 1) * T, :])
            for u in range(t, nt):
                tiles[u, j] = st[(u - t) * T:(u - t + 1) * T]
        for t in range(nt):
            jd = nfull - 1 + t
            tiles[t, jd] = jnp.where(causal, tiles[t, jd], MASK_VAL)
        return tiles

    def softmax_pv(i, tiles):
        r0 = i * BQ
        nfull = r0 // T + 1
        for t in range(nt):
            nk = nfull + t
            mx = tiles[t, 0]
            for j in range(1, nk):
                mx = jnp.maximum(mx, tiles[t, j])
            m = jnp.max(mx, axis=1, keepdims=True)
            lacc = o = None
            cj = ACK // T
            for j0 in range(0, nk, cj):
                ps = []
                for j in range(j0, min(nk, j0 + cj)):
                    p = jnp.exp2(tiles[t, j] - m)
                    lacc = p if lacc is None else lacc + p
                    ps.append(p)
                pc = jnp.concatenate(ps, axis=1) if len(ps) > 1 else ps[0]
                oo = _dot(pc.astype(BF16), v_s[h, j0 * T:(j0 + len(ps)) * T, :])
                o = oo if o is None else o + oo
            l = jnp.sum(lacc, axis=1, keepdims=True)
            o_s[ho, r0 + t * T:r0 + (t + 1) * T, :] = (
                o * pl.reciprocal(l, approx=True)).astype(BF16)

    order = list(range(nblk - 1, -1, -1))
    pend = []
    for a in range(nblk + ADEPTH):
        if a < nblk:
            pend.append(scores(order[a]))
        if a >= ADEPTH:
            softmax_pv(order[a - ADEPTH], pend.pop(0))


HS = S // 2


def _lhs_sums(a11, a12, a21, a22):
    return (a11 + a22, a21 + a22, a11 + a12, a21 - a11, a12 - a22)


def _rhs_ops(b11, b12, b21, b22):
    return (b11 + b22, b11, b12 - b22, b21 - b11, b22, b11 + b12, b21 + b22)


def _strassen(lhs, rhs):
    m1, m2, m3, m4, m5, m6, m7 = [_dot(a, b) for a, b in zip(lhs, rhs)]
    return (((m1 + m4) - m5) + m7, m3 + m5, m2 + m4, ((m1 - m2) + m3) + m6)


PR = 256
OR = 128
BR = 512
DSUB = 64
P2D = 1
P2U = 4
WSL = 16
WSL2 = 32
OCH = 1
OVAR = 0
AREP = 1
DMA_A = 20
DMA_B = 32
PORD = 3
WORD = 3
NWO = 16


def _kernel(ax_hbm, ac_hbm, wq_hbm, wuk_hbm, wuv_hbm, wo_hbm, bx_hbm, wrT_hbm, wiT_hbm,
            gdf_hbm, gnf_hbm, gdi_hbm, gni_hbm, gsf_hbm, gsi_hbm,
            out_hbm,
            ax_s, ac_s, w_st, wo_s, zs_s, gdi_s, gni_s, sems, wosem, xsem):
    def copy(src, dst, i):
        return pltpu.make_async_copy(src, dst, sems.at[i])

    def wcopies(g):
        hs = pl.ds(pl.multiple_of(g * 8, 8), 8)
        return (copy(wq_hbm.at[:, hs, :], w_st.at[pl.ds(0, DM)], 2),
                copy(wuk_hbm.at[:, hs, :], w_st.at[pl.ds(DM, DC)], 3),
                copy(wuv_hbm.at[:, hs, :], w_st.at[pl.ds(DM + DC, DC)], 4))

    def wocopies(u):
        r = pl.multiple_of(u * T, T)
        r2 = pl.multiple_of(H * HD // 2 + u * T, T)
        return (pltpu.make_async_copy(wo_hbm.at[pl.ds(r, T), :], wo_s.at[pl.ds(r, T), :], wosem.at[2 * u]),
                pltpu.make_async_copy(wo_hbm.at[pl.ds(r2, T), :], wo_s.at[pl.ds(r2, T), :], wosem.at[2 * u + 1]))

    def xcopies(u):
        r = pl.multiple_of(u * T, T)
        r2 = pl.multiple_of(HS + u * T, T)
        return (pltpu.make_async_copy(ax_hbm.at[pl.ds(r, T), :], ax_s.at[pl.ds(r, T), :], xsem.at[2 * u]),
                pltpu.make_async_copy(ax_hbm.at[pl.ds(r2, T), :], ax_s.at[pl.ds(r2, T), :], xsem.at[2 * u + 1]))

    def prep_lhs(src, dst, i):
        kk = src.shape[1] // 2
        for a in range(0, T, WSL):
            r = pl.multiple_of(i * T + a, WSL)
            top = src[pl.ds(r, WSL), :].astype(F32)
            bot = src[pl.ds(HS + r, WSL), :].astype(F32)
            ops = [v.astype(BF16) for v in _lhs_sums(top[:, :kk], top[:, kk:], bot[:, :kk], bot[:, kk:])]
            for j in range(5):
                dst[j, pl.ds(r, WSL), :] = ops[j]
            src[S:S + 16, 0:T] = ops[4][0:16, 0:T]

    def b_phase(xs_s, cs_s, bx_s, y_s, wrT_s, wiT_s, wd_s, wt_s, xre_s, xim_s, ys_s,
                gdf_s, gnf_s, gsf_s, gsi_s, bsem):
        def bcopy(src, dst, i):
            return pltpu.make_async_copy(src, dst, bsem.at[i])
        nch = S // BR
        xc = [bcopy(bx_hbm.at[pl.ds(i * BR, BR), :], bx_s.at[pl.ds(i * BR, BR), :], i)
              for i in range(nch)]
        cc = [bcopy(gdf_hbm, gdf_s, nch), bcopy(gnf_hbm, gnf_s, nch + 1),
              bcopy(wrT_hbm, wrT_s, nch + 2), bcopy(wiT_hbm, wiT_s, nch + 3),
              bcopy(gsf_hbm, gsf_s, nch + 4), bcopy(gsi_hbm, gsi_s, nch + 5)]
        xc[0].start()
        cc[0].start()
        cc[1].start()
        xc[1].start()

        cc[0].wait()
        cc[1].wait()
        xc[0].wait()
        xc[2].start()
        _b_d_forward_vpu(bx_s, y_s, 0, 0, BR)

        def dfwd(i, c):
            r1 = pl.multiple_of((i + 1) * BR, BR)
            bcopy(bx_hbm.at[pl.ds(r1, BR), :], bx_s.at[pl.ds(r1, BR), :], i + 1).wait()

            @pl.when(i == 0)
            def _():
                xc[3].start()

            @pl.when(i == 2)
            def _():
                cc[2].start()
                cc[3].start()
            for a in range(0, BR, DSUB):
                _b_d_forward_mxu(y_s, i % 2, gdf_s, gnf_s, xre_s, xim_s,
                                 pl.multiple_of(i * BR, BR), a, DSUB)
                for b in range(a, a + DSUB, VSL):
                    _b_d_forward_vpu_slab(bx_s, y_s, (i + 1) % 2, r1, b)
            return c
        lax.fori_loop(0, nch - 1, dfwd, 0)
        for a in range(0, BR, DSUB):
            _b_d_forward_mxu(y_s, (nch - 1) % 2, gdf_s, gnf_s, xre_s, xim_s, (nch - 1) * BR, a, DSUB)

        cc[2].wait()
        cc[3].wait()
        cc[4].start()
        cc[5].start()
        copy(ac_hbm, ac_s.at[pl.ds(0, S)], 1).start()

        def p1(i, c):
            @pl.when(i == 2)
            def _():
                for u in range(8):
                    for cp in xcopies(u):
                        cp.start()

            @pl.when(i == 6)
            def _():
                for cp in wcopies(0):
                    cp.start()
            for v in range(NCT):
                u = i * NCT + v
                _b_s_pass1(xre_s, xim_s, ys_s, u // 8, u % 8)
            for v in range(2):
                _b_prepare_w(wrT_s, wiT_s, wd_s, wt_s, 2 * i + v)
            return c
        lax.fori_loop(0, 8, p1, 0)
        cc[4].wait()
        cc[5].wait()
        copy(ac_hbm, ac_s.at[pl.ds(0, S)], 1).wait()

        def p2(kk, c):
            for cp in xcopies(kk):
                cp.wait()

            @pl.when((kk >= 2) & (kk < 2 + 4))
            def _():
                for v in range(NWO // 4):
                    for cp in wocopies((kk - 2) * (NWO // 4) + v):
                        cp.start()

            @pl.when(kk == 7)
            def _():
                copy(gdi_hbm, gdi_s, 8).start()
                copy(gni_hbm, gni_s, 9).start()
            _b_s_pass2(ys_s, zs_s, wt_s, gsf_s, gsi_s, [kk * P2U + u for u in range(P2U)])
            prep_lhs(ac_s, cs_s, kk)
            prep_lhs(ax_s, xs_s, kk)
            return c
        lax.fori_loop(0, N1 // P2U, p2, 0)

    def b_scope(xs_s, cs_s):
      pl.run_scoped(
        functools.partial(b_phase, xs_s, cs_s),
        pltpu.VMEM((S, DM), BF16), pltpu.VMEM((2, BR, DM), BF16),
        pltpu.VMEM((DF, S), BF16), pltpu.VMEM((DF, S), BF16),
        pltpu.VMEM((S // T, 512, T), U32), pltpu.VMEM((NCT, S, T), U32),
        pltpu.VMEM((NCT, S, T), F32), pltpu.VMEM((NCT, S, T), F32),
        pltpu.VMEM((N1, NCT, T, T), BF16),
        pltpu.VMEM((4, 256, 256), BF16), pltpu.VMEM((T, T), BF16),
        pltpu.VMEM((N1, T, T), BF16), pltpu.VMEM((N1, T, T), BF16),
        pltpu.SemaphoreType.DMA((S // BR + 6,)),
    )

    def a_outer(ctx_s, wos_s):
        def a_main(xs_s, cs_s, wu_s, q_s, k_s, v_s):
            def stage_w(i, chain):
                rows = (DM + 2 * DC) // 8
                step = WSL2 if chain else 128
                for a in range(0, rows, step):
                    r = pl.multiple_of(i * rows + a, step)
                    v = w_st[pl.ds(r, step)]
                    wu_s[pl.ds(pl.multiple_of(4 * r, 4 * step), 4 * step), :] = pltpu.bitcast(
                        v.reshape(step * 8, HD), U32)
                    if chain:
                        w_st[DM + 2 * DC:DM + 2 * DC + 2] = v[0:2]

            def w_rhs(slot, base, kk):
                def blk(m0, hp0):
                    cols = []
                    for hp in (hp0, hp0 + 1):
                        x = wu_s[pl.ds(4 * m0 + hp, kk, stride=4), :]
                        cols.append(pltpu.bitcast(x << 16, F32))
                        cols.append(pltpu.bitcast(x & jnp.uint32(0xFFFF0000), F32))
                    return jnp.concatenate(cols, axis=1)
                b11, b12 = blk(base, 0), blk(base, 2)
                b21, b22 = blk(base + kk, 0), blk(base + kk, 2)
                return [v.astype(BF16) for v in _rhs_ops(b11, b12, b21, b22)]

            def prep_wo(u, chain):
                step = WSL if chain else T
                for a in range(0, T, step):
                    r = pl.multiple_of(u * T + a, step)
                    top = wo_s[pl.ds(r, step), :].astype(F32)
                    bot = wo_s[pl.ds(H * HD // 2 + r, step), :].astype(F32)
                    ops = _rhs_ops(top[:, :512], top[:, 512:], bot[:, :512], bot[:, 512:])
                    for jj, j in enumerate((0, 2, 3, 5, 6)):
                        v = ops[j].astype(BF16)
                        wos_s[jj, pl.ds(r, step), :] = v
                    if chain:
                        wo_s[H * HD:H * HD + 16, 0:HD] = v[0:16, 0:HD]

            for cp in wcopies(0):
                cp.wait()

            def prew(i, c):
                stage_w(i, False)
                return c
            lax.fori_loop(0, 8, prew, 0)

            def lhs7(src, sums, r):
                kk = src.shape[1] // 2
                top, bot = pl.ds(r, PR), pl.ds(HS + r, PR)
                return (sums[0, top, :], sums[1, top, :], src[top, :kk], src[bot, kk:],
                        sums[2, top, :], sums[3, top, :], sums[4, top, :])

            def group(g, c):
                slot = 0
                gn = jnp.minimum(g + 1, NG - 1)
                for cp in wcopies(gn):
                    cp.start()

                def chunk(i, cc):
                    r = pl.multiple_of(i * PR, PR)
                    top, bot = pl.ds(r, PR), pl.ds(HS + r, PR)
                    for cp in wocopies(g * 4 + i):
                        cp.wait()

                    def put(dst, cs, scale=None):
                        for cb, rows, h0 in zip(cs, (top, top, bot, bot), (0, 4, 0, 4)):
                            if scale is not None:
                                cb = cb * scale
                            cb = cb.astype(BF16)
                            for hh in range(4):
                                dst[h0 + hh, rows, :] = cb[:, hh * HD:(hh + 1) * HD]
                    cl = lhs7(ac_s, cs_s, r)
                    put(k_s, _strassen(cl, w_rhs(slot, DM, DC // 2)))
                    put(v_s, _strassen(cl, w_rhs(slot, DM + DC, DC // 2)))
                    put(q_s, _strassen(lhs7(ax_s, xs_s, r), w_rhs(slot, 0, DM // 2)), Q_SCALE)
                    if WORD < 9: prep_wo(g * 4 + i, True)
                    return cc
                lax.fori_loop(0, HS // PR, chunk, 0)

                for cp in wcopies(gn):
                    cp.wait()

                def head(h, cc):
                    _attn_head(q_s, k_s, v_s, ctx_s, h, g * 8 + h)
                    if PORD < 9: stage_w(h, True)
                    return cc
                lax.fori_loop(0, 8, head, 0)
                return c
            lax.fori_loop(0, NG, group, 0)

        def lhs_scope(xs_s, cs_s):
            b_scope(xs_s, cs_s)
            pl.run_scoped(functools.partial(a_main, xs_s, cs_s),
                          pltpu.VMEM((4 * (DM + 2 * DC), HD), U32),
                          *[pltpu.VMEM((8, S, HD), BF16)] * 3)

        pl.run_scoped(lhs_scope,
                      pltpu.VMEM((5, HS, DM // 2), BF16), pltpu.VMEM((5, HS, DC // 2), BF16))

        def a_out(oa_s, yb_s, xre_s, xim_s, ls_s, osem):
            nch = HS // OR

            def ocopies(i):
                r = pl.multiple_of(i * OR, OR)
                r2 = pl.multiple_of(HS + i * OR, OR)
                return (pltpu.make_async_copy(oa_s.at[pl.ds(r, OR), :],
                                              out_hbm.at[pl.ds(r, OR), pl.ds(0, DM)], osem.at[2 * i]),
                        pltpu.make_async_copy(oa_s.at[pl.ds(r2, OR), :],
                                              out_hbm.at[pl.ds(r2, OR), pl.ds(0, DM)], osem.at[2 * i + 1]))

            def ycopy(i):
                r = pl.multiple_of(i * BR, BR)
                return pltpu.make_async_copy(yb_s.at[pl.ds(r, BR), :],
                                             out_hbm.at[pl.ds(r, BR), pl.ds(DM, DM)], osem.at[2 * nch + i])

            def blk(rows, h0):
                return [ctx_s[h0 + h, rows, :] for h in range(H // 2)]

            def ochunk(i, c):
                r = pl.multiple_of(i * OR, OR)
                top, bot = pl.ds(r, OR), pl.ds(HS + r, OR)
                cat = lambda xs: jnp.concatenate(xs, axis=1)
                hk = H * HD // 2
                a11, a22 = cat(blk(top, 0)), cat(blk(bot, 16))
                m3 = _dot(a11, wos_s[1])
                m4 = _dot(a22, wos_s[2])
                if OVAR == 0:
                    a12, a21 = cat(blk(top, 16)), cat(blk(bot, 0))
                    sums = [v.astype(BF16) for v in
                            _lhs_sums(*[v.astype(F32) for v in (a11, a12, a21, a22)])]
                else:
                    for h in range(H // 2):
                        ops = _lhs_sums(ctx_s[h, top, :].astype(F32), ctx_s[16 + h, top, :].astype(F32),
                                        ctx_s[h, bot, :].astype(F32), ctx_s[16 + h, bot, :].astype(F32))
                        ops = [v.astype(BF16) for v in ops]
                        for j in range(5):
                            ls_s[j, :, h * HD:(h + 1) * HD] = ops[j]
                    sums = [ls_s[j] for j in range(5)]
                m1 = _dot(sums[0], wos_s[0])
                m2 = _dot(sums[1], wo_s[0:hk, 0:512])
                m5 = _dot(sums[2], wo_s[hk:2 * hk, 512:1024])
                m6 = _dot(sums[3], wos_s[3])
                m7 = _dot(sums[4], wos_s[4])
                cs = (((m1 + m4) - m5) + m7, m3 + m5, m2 + m4, ((m1 - m2) + m3) + m6)
                for cb, rows, c0 in zip(cs, (top, top, bot, bot), (0, 512, 0, 512)):
                    oa_s[rows, c0:c0 + 512] = cb.astype(BF16)
                for cp in ocopies(i):
                    cp.start()
                for v in range(NCT * 8 // nch):
                    u = i * (NCT * 8 // nch) + v
                    _b_s_pass3(zs_s, xre_s, xim_s, u // 8, u % 8, True)
                return c
            lax.fori_loop(0, nch, ochunk, 0)

            copy(gdi_hbm, gdi_s, 8).wait()
            copy(gni_hbm, gni_s, 9).wait()

            def dinv(i, c):
                _b_d_inverse(xre_s, xim_s, gdi_s, gni_s, yb_s, pl.multiple_of(i * BR, BR), BR)
                ycopy(i).start()
                return c
            lax.fori_loop(0, S // BR, dinv, 0)
            for i in range(nch):
                for cp in ocopies(i):
                    cp.wait()
            for i in range(S // BR):
                ycopy(i).wait()

        pl.run_scoped(a_out, pltpu.VMEM((S, DM), BF16), pltpu.VMEM((S, DM), BF16),
                      pltpu.VMEM((NCT, S, T), F32), pltpu.VMEM((NCT, S, T), F32),
                      pltpu.VMEM((5, OR, H * HD // 2), BF16),
                      pltpu.SemaphoreType.DMA((2 * (HS // OR) + S // BR,)))

    pl.run_scoped(a_outer, pltpu.VMEM((H + 1, S, HD), BF16), pltpu.VMEM((5, H * HD // 2, 512), BF16))


@jax.jit
def pallas_concat_heads__compressed_kv_cla__spectral_gfnet__prompt_kernel(
    A_x, A_c_kv, A_w_q, A_w_uk, A_w_uv, A_w_o, B_x, B_w_r, B_w_i,
):
    hbm = pl.BlockSpec(memory_space=pl.ANY)
    out = pl.pallas_call(
        _kernel,
        in_specs=[hbm] * 15,
        out_specs=hbm,
        out_shape=jax.ShapeDtypeStruct((S, 2 * DM), BF16),
        scratch_shapes=[
            pltpu.VMEM((S + 16, DM), BF16), pltpu.VMEM((S + 16, DC), BF16),
            pltpu.VMEM((DM + 2 * DC + 2, 8, HD), BF16),
            pltpu.VMEM((H * HD + 16, DM), BF16),
            pltpu.VMEM((N1 + 1, NCT, T, T), BF16),
            pltpu.VMEM((4, 256, 256), BF16), pltpu.VMEM((T, T), BF16),
            pltpu.SemaphoreType.DMA((10,)), pltpu.SemaphoreType.DMA((2 * NWO,)),
            pltpu.SemaphoreType.DMA((16,)),
        ],
        compiler_params=pltpu.CompilerParams(vmem_limit_bytes=120 * 1024 * 1024),
    )(A_x.reshape(S, DM), A_c_kv.reshape(S, DC), A_w_q, A_w_uk, A_w_uv,
      A_w_o.reshape(H * HD, DM), B_x.reshape(S, DM), B_w_r.T, B_w_i.T, *_CONSTS)
    return out.reshape(1, S, 2 * DM)
```

```python
import functools
import math

import jax
import jax.numpy as jnp
import numpy as np
from jax import lax
from jax.experimental import pallas as pl
from jax.experimental.pallas import tpu as pltpu

S = 2048
DM = 1024
DC = 512
H = 32
HD = 128
T = 128
NG = 4
DF = DM // 2 + 1
NCT = 5
N1, N2 = 32, 64

F32, BF16, U32 = jnp.float32, jnp.bfloat16, jnp.uint32
LOG2E = math.log2(math.e)
Q_SCALE = float(HD ** -0.5 * LOG2E)
MASK_VAL = float(-1e9 * LOG2E)
CLASS_PAIRS = ((0, 4), (1, 7), (2, 6), (3, 5))


def _make_constants():
    b = np.arange(128)[:, None].astype(np.float64)
    m = np.arange(64)[None, :].astype(np.float64)

    def cs(r):
        th = 2.0 * np.pi * b * (r + 8.0 * m) / DM
        return np.cos(th), np.sin(th)

    gdf = np.zeros((4, 256, 256))
    c0, s0 = cs(0)
    c4, s4 = cs(4)
    gdf[0, :128, 0:64], gdf[0, :128, 128:192] = c0, -s0
    gdf[0, 128:, 64:128], gdf[0, 128:, 192:256] = c4, -s4
    for p in (1, 2, 3):
        r, r2 = CLASS_PAIRS[p]
        c, s = cs(r)
        c2, s2 = cs(r2)
        gdf[p, :128, 0:64], gdf[p, 128:, 0:64] = c, s
        gdf[p, :128, 64:128], gdf[p, 128:, 64:128] = c2, -s2
        gdf[p, :128, 128:192], gdf[p, 128:, 128:192] = -s, c
        gdf[p, :128, 192:256], gdf[p, 128:, 192:256] = -s2, -c2
    alt = (-1.0) ** np.arange(128)
    gnf = np.zeros((128, 128))
    gnf[:, 0] = alt

    sc = 1.0 / (S * DM)
    gdi = np.zeros((4, 256, 256))
    w0 = np.full((64, 1), 2.0)
    w0[0] = 1.0
    gdi[0, 0:64, 0:128] = (c0.T * w0) * sc
    gdi[0, 128:192, 0:128] = (-s0.T * w0) * sc
    gdi[0, 128, :] = 0.0
    gdi[0, 64:128, 128:256] = 2.0 * c4.T * sc
    gdi[0, 192:256, 128:256] = -2.0 * s4.T * sc
    for p in (1, 2, 3):
        r, r2 = CLASS_PAIRS[p]
        c, s = cs(r)
        c2, s2 = cs(r2)
        f = 2.0 * sc
        gdi[p, 0:64, 0:128], gdi[p, 128:192, 0:128] = f * c.T, -f * s.T
        gdi[p, 64:128, 0:128], gdi[p, 192:256, 0:128] = f * c2.T, -f * s2.T
        gdi[p, 0:64, 128:256], gdi[p, 128:192, 128:256] = f * s.T, f * c.T
        gdi[p, 64:128, 128:256], gdi[p, 192:256, 128:256] = -f * s2.T, -f * c2.T
    gni = np.zeros((128, 128))
    gni[0, :] = alt * sc

    n2 = np.arange(N2)
    perm = np.concatenate([np.concatenate([8 * j + np.arange(8), 64 + 8 * j + np.arange(8)])
                           for j in range(8)])
    gsf = np.zeros((N1, 128, 128))
    gsi = np.zeros((N1, 128, 128))
    for k1 in range(N1):
        k = k1 + N1 * n2
        g = np.exp(-2j * np.pi * np.outer(k, n2) / S)
        ghat = np.block([[g.real, -g.imag], [g.imag, g.real]])
        gsf[k1] = ghat[perm][:, perm]
        gsi[k1] = ghat.T[perm][:, perm]
    def words(a):
        u = np.asarray(a, dtype=np.float32).astype(jnp.bfloat16).view(np.uint16).astype(np.uint32)
        return np.ascontiguousarray(u[..., 0::2, :] | (u[..., 1::2, :] << 16))
    return tuple(words(a) for a in (gdf, gnf, gdi, gni, gsf, gsi))


_CONSTS = _make_constants()


def _dot(a, b):
    return jnp.dot(a, b, preferred_element_type=F32)


def _dot_nt(a, b):
    return lax.dot_general(a, b, (((1,), (1,)), ((), ())), preferred_element_type=F32)


def _ld(ref, *idx):
    return pltpu.bitcast(ref[idx], BF16)


def _pk(v):
    return pltpu.bitcast(v.astype(BF16), U32)


def _rows(r0, n):
    return pl.ds(r0 // 2, n // 2)


def _cmul_const(x, e, n, sign):
    re, im = x
    e %= n
    if e == 0:
        return re, im
    if 8 * e % n == 0:
        o = 8 * e // n
        if sign < 0:
            o = (8 - o) % 8
        h = math.sqrt(0.5)
        if o == 2:
            return -im, re
        if o == 4:
            return -re, -im
        if o == 6:
            return im, -re
        if o == 1:
            return (re - im) * h, (re + im) * h
        if o == 3:
            return (re + im) * (-h), (re - im) * h
        if o == 5:
            return (im - re) * h, (re + im) * (-h)
        if o == 7:
            return (re + im) * h, (im - re) * h
    th = sign * 2.0 * math.pi * e / n
    c, s = math.cos(th), math.sin(th)
    return re * c - im * s, re * s + im * c


def _cadd(a, b):
    return a[0] + b[0], a[1] + b[1]


def _csub(a, b):
    return a[0] - b[0], a[1] - b[1]


def _fft(xs, sign):
    n = len(xs)
    if n == 1:
        return xs
    if n == 2:
        return [_cadd(xs[0], xs[1]), _csub(xs[0], xs[1])]
    u = _fft(xs[0::2], sign)
    z1 = _fft(xs[1::4], sign)
    z3 = _fft(xs[3::4], sign)
    out = [None] * n
    q = n // 4
    for k in range(q):
        a = _cmul_const(z1[k], k, n, sign)
        b = _cmul_const(z3[k], 3 * k, n, sign)
        sm, df = _cadd(a, b), _csub(a, b)
        out[k] = _cadd(u[k], sm)
        out[k + 2 * q] = _csub(u[k], sm)
        if sign < 0:
            out[k + q] = (u[k + q][0] + df[1], u[k + q][1] - df[0])
            out[k + 3 * q] = (u[k + q][0] - df[1], u[k + q][1] + df[0])
        else:
            out[k + q] = (u[k + q][0] - df[1], u[k + q][1] + df[0])
            out[k + 3 * q] = (u[k + q][0] + df[1], u[k + q][1] - df[0])
    return out


def _b_prepare_w(wrT_s, wiT_s, wd_s, wt_s, t):
    def words(a, b):
        return (pltpu.bitcast(a.astype(F32), U32) >> 16) | (
            pltpu.bitcast(b.astype(F32), U32) & jnp.uint32(0xFFFF0000))

    rows = pl.ds(pl.multiple_of(t * T, T), T)
    for a in range(0, 512, 64):
        wd_s[t, a:a + 64, :] = words(wrT_s[a:a + 64, rows], wiT_s[a:a + 64, rows])
    for p, (r, r2) in enumerate(CLASS_PAIRS):
        a = wd_s[t, pl.ds(r, 64, stride=8), :]
        b = wd_s[t, pl.ds(r2, 64, stride=8), :]
        wt_s[p, rows, :] = jnp.concatenate([a, b], axis=0).T
    ny = words(wrT_s[512:513, rows], wiT_s[512:513, rows])
    row = lax.broadcasted_iota(jnp.int32, (T, T), 0)
    wt_s[4, rows, :] = jnp.where(row == 0, jnp.broadcast_to(ny, (T, T)), jnp.uint32(0)).T


def _b_d_forward_vpu(xb_s, y_s, slot, r0, rows):
    for a in range(0, rows, VSL):
        _b_d_forward_vpu_slab(xb_s, y_s, slot, r0, a)


def _b_d_forward_vpu_slab(xb_s, y_s, slot, r0, a):
    sl = pl.ds(r0 + a, VSL)
    x = [xb_s[sl, a * T:(a + 1) * T].astype(F32) for a in range(8)]
    s04, t = x[0] + x[4], x[0] - x[4]
    s26, u = x[2] + x[6], x[2] - x[6]
    s15, v = x[1] + x[5], x[1] - x[5]
    s37, w = x[3] + x[7], x[3] - x[7]
    e, f = s04 + s26, s04 - s26
    g, hh = s15 + s37, s15 - s37
    k = math.sqrt(0.5)
    al, be = (v - w) * k, (v + w) * k
    ys = ((e + g, e - g),
          (t + al, -(u + be)),
          (f, -hh),
          (t - al, u - be))
    for p in range(4):
        y_s[slot, a // 2:(a + VSL) // 2, 2 * p * T:(2 * p + 2) * T] = _pk(jnp.concatenate(
            [ys[p][0], ys[p][1]], axis=1))


def _b_d_forward_mxu(y_s, slot, gdf_s, gnf_s, xre_s, xim_s, r0, a, rows):
    sl = pl.ds(r0 + a, rows)
    for p in range(4):
        o = _dot(_ld(y_s, slot, slice(a // 2, (a + rows) // 2), slice(2 * p * T, (2 * p + 2) * T)), _ld(gdf_s, p))
        xre_s[p, sl, :] = o[:, :T]
        xim_s[p, sl, :] = o[:, T:]
    xre_s[4, sl, :] = _dot(_ld(y_s, slot, slice(a // 2, (a + rows) // 2), slice(0, T)),
                           pltpu.bitcast(gnf_s[...], BF16))
    xim_s[4, sl, :] = jnp.zeros((rows, T), F32)


def _fft32(load, emit, sign):
    half = N1 // 2
    for par in range(2):
        xs = []
        for n in range(half):
            a, b = load(n), load(n + half)
            xs.append(_cadd(a, b) if par == 0 else _cmul_const(_csub(a, b), n, N1, sign))
        out = _fft(xs, sign)
        for q in range(half):
            emit(2 * q + par, out[q])


def _b_s_pass1(xre_s, xim_s, ys_s, c, j):
    off = pl.multiple_of(j * 8, 8)

    def load(n1):
        rows = pl.ds(N2 * n1 + off, 8)
        return xre_s[c, rows, :], xim_s[c, rows, :]

    def emit(k1, v):
        ys_s[k1, c, pl.ds(pl.multiple_of(j * 16, 16), 16), :] = jnp.concatenate(v, axis=0).astype(BF16)
    _fft32(load, emit, -1)


def _b_s_pass2_fwd(ys_s, gsf_s, k1):
    rhs = jnp.concatenate([ys_s[k1, c] for c in range(NCT)], axis=1)
    return _dot(_ld(gsf_s, k1), rhs)


def _b_s_pass2_inv(vv, zs_s, wt_s, gsi_s, k1):
    outs = []
    for c in range(NCT):
        wd = wt_s[c, pl.ds(k1, N2, stride=N1), :]
        wr = pltpu.bitcast(wd << 16, F32)
        wi = pltpu.bitcast(wd & jnp.uint32(0xFFFF0000), F32)
        pcs = []
        for j in range(8):
            vr = vv[16 * j:16 * j + 8, c * T:(c + 1) * T]
            vi = vv[16 * j + 8:16 * j + 16, c * T:(c + 1) * T]
            a, b = wr[8 * j:8 * j + 8], wi[8 * j:8 * j + 8]
            pcs.append(vr * a - vi * b)
            pcs.append(vr * b + vi * a)
        outs.append(jnp.concatenate(pcs, axis=0).astype(BF16))
    ginv = _ld(gsi_s, k1)
    for c in range(NCT):
        zs_s[k1, c] = _dot(ginv, outs[c]).astype(BF16)


def _b_s_pass2(ys_s, zs_s, wt_s, gsf_s, gsi_s, k1s):
    pend = []
    for a in range(len(k1s) + P2D):
        if a < len(k1s):
            pend.append(_b_s_pass2_fwd(ys_s, gsf_s, k1s[a]))
        if a >= P2D:
            _b_s_pass2_inv(pend.pop(0), zs_s, wt_s, gsi_s, k1s[a - P2D])


def _b_s_pass3(zs_s, xre_s, xim_s, c, j, chain):
    off = pl.multiple_of(j * 8, 8)

    def load(k1):
        z = zs_s[k1, c, pl.ds(pl.multiple_of(j * 16, 16), 16), :].astype(F32)
        return z[0:8], z[8:16]

    def emit(n1, v):
        rows = pl.ds(N2 * n1 + off, 8)
        xre_s[c, rows, :] = v[0]
        xim_s[c, rows, :] = v[1]
        if chain and n1 >= N1 - 2:
            zs_s[N1, 0, 0:16, :] = jnp.concatenate(v, axis=0).astype(BF16)
    _fft32(load, emit, +1)


def _b_d_inverse(xre_s, xim_s, gdi_s, gni_s, yb_s, r0, rows):
    sl = pl.ds(r0, rows)
    us = []
    for p in range(4):
        lhs = jnp.concatenate([xre_s[p, sl, :], xim_s[p, sl, :]], axis=1).astype(BF16)
        o = _dot(lhs, _ld(gdi_s, p))
        us.append((o[:, :T], o[:, T:]))
    u0 = us[0][0] + _dot(xre_s[4, sl, :].astype(BF16), pltpu.bitcast(gni_s[...], BF16))
    u4 = us[0][1]
    (u1r, u1i), (u2r, u2i), (u3r, u3i) = us[1], us[2], us[3]
    e0, e1 = u0 + u4, u0 - u4
    ev = (e0 + u2r, e1 - u2i, e0 - u2r, e1 + u2i)
    pq, qq = u1r - u3r, u1i + u3i
    k = math.sqrt(0.5)
    od = (u1r + u3r, (pq - qq) * k, u3i - u1i, (pq + qq) * (-k))
    for a in range(4):
        yb_s[sl, a * T:(a + 1) * T] = (ev[a] + od[a]).astype(BF16)
        yb_s[sl, (a + 4) * T:(a + 5) * T] = (ev[a] - od[a]).astype(BF16)


VSL = 16
BQ = 128
ADEPTH = 2
ACK = 128
AORD = 2
AUN = 2


def _attn_order(h0):
    n = S // BQ
    if AORD == 0:
        return [(h0 + u, i) for u in range(AUN) for i in range(n - 1, -1, -1)]
    if AORD == 1:
        return [p for i in range(n) for p in ((h0, n - 1 - i), (h0 + 1, i))]
    if AORD == 2:
        o = []
        lo, hi = 0, n - 1
        while lo <= hi:
            o.append(hi)
            hi -= 1
            if lo <= hi:
                o.append(lo)
                lo += 1
        return [(h0 + u, i) for u in range(AUN) for i in o]


def _attn_heads(q_s, k_s, v_s, o_s, h0, ho):
    nt = BQ // T
    row = lax.broadcasted_iota(jnp.int32, (T, T), 0)
    col = lax.broadcasted_iota(jnp.int32, (T, T), 1)
    causal = col <= row

    def scores(h, i):
        r0 = i * BQ
        nfull = r0 // T + 1
        tiles = {}
        s = _dot_nt(_ld(q_s, h, _rows(r0, BQ)), _ld(k_s, h, _rows(0, nfull * T)))
        for t in range(nt):
            for j in range(nfull):
                tiles[t, j] = s[t * T:(t + 1) * T, j * T:(j + 1) * T]
        for t in range(1, nt):
            j = nfull - 1 + t
            st = _dot_nt(_ld(q_s, h, _rows(r0 + t * T, BQ - t * T)), _ld(k_s, h, _rows(j * T, T)))
            for u in range(t, nt):
                tiles[u, j] = st[(u - t) * T:(u - t + 1) * T]
        for t in range(nt):
            jd = nfull - 1 + t
            tiles[t, jd] = jnp.where(causal, tiles[t, jd], MASK_VAL)
        return tiles

    def softmax_pv(h, i, tiles):
        r0 = i * BQ
        nfull = r0 // T + 1
        for t in range(nt):
            nk = nfull + t
            mx = tiles[t, 0]
            for j in range(1, nk):
                mx = jnp.maximum(mx, tiles[t, j])
            m = jnp.max(mx, axis=1, keepdims=True)
            lacc = o = None
            cj = ACK // T
            for j0 in range(0, nk, cj):
                ps = []
                for j in range(j0, min(nk, j0 + cj)):
                    p = jnp.exp2(tiles[t, j] - m)
                    lacc = p if lacc is None else lacc + p
                    ps.append(p)
                pc = jnp.concatenate(ps, axis=1) if len(ps) > 1 else ps[0]
                oo = _dot(pc.astype(BF16), _ld(v_s, h, _rows(j0 * T, len(ps) * T)))
                o = oo if o is None else o + oo
            l = jnp.sum(lacc, axis=1, keepdims=True)
            o_s[h - h0 + ho, _rows(r0 + t * T, T)] = _pk(o * pl.reciprocal(l, approx=True))

    order = _attn_order(h0)
    pend = []
    for a in range(len(order) + ADEPTH):
        if a < len(order):
            pend.append(scores(*order[a]))
        if a >= ADEPTH:
            softmax_pv(*order[a - ADEPTH], pend.pop(0))


HS = S // 2


def _lhs_sums(a11, a12, a21, a22):
    return (a11 + a22, a21 + a22, a11 + a12, a21 - a11, a12 - a22)


def _rhs_ops(b11, b12, b21, b22):
    return (b11 + b22, b11, b12 - b22, b21 - b11, b22, b11 + b12, b21 + b22)


def _strassen(lhs, rhs):
    m1, m2, m3, m4, m5, m6, m7 = [_dot(a, b) for a, b in zip(lhs, rhs)]
    return (((m1 + m4) - m5) + m7, m3 + m5, m2 + m4, ((m1 - m2) + m3) + m6)


PR = 256
OR = 128
BR = 512
DSUB = 64
P2D = 1
P2U = 8
WSL = 16
WSL2 = 32
OCH = 1
AREP = 1
DMA_A = 4
DMA_B = 32
P1ORD = 0
PORD = 3
WORD = 3
NWO = 16


def _kernel(ax_hbm, ac_hbm, wq_hbm, wuk_hbm, wuv_hbm, wo_hbm, bx_hbm, wrT_hbm, wiT_hbm,
            gdf_hbm, gnf_hbm, gdi_hbm, gni_hbm, gsf_hbm, gsi_hbm,
            out_hbm,
            ax_s, ac_s, w_st, wo_s, zs_s, gdi_s, gni_s, sems, wosem):
    def copy(src, dst, i):
        return pltpu.make_async_copy(src, dst, sems.at[i])

    def wcopies(g):
        hs = pl.ds(pl.multiple_of(g * 8, 8), 8)
        return (copy(wq_hbm.at[:, hs, :], w_st.at[pl.ds(0, DM)], 2),
                copy(wuk_hbm.at[:, hs, :], w_st.at[pl.ds(DM, DC)], 3),
                copy(wuv_hbm.at[:, hs, :], w_st.at[pl.ds(DM + DC, DC)], 4))

    def wocopies(u):
        r = pl.multiple_of(u * T, T)
        r2 = pl.multiple_of(H * HD // 2 + u * T, T)
        return (pltpu.make_async_copy(wo_hbm.at[pl.ds(r, T), :], wo_s.at[pl.ds(r, T), :], wosem.at[2 * u]),
                pltpu.make_async_copy(wo_hbm.at[pl.ds(r2, T), :], wo_s.at[pl.ds(r2, T), :], wosem.at[2 * u + 1]))

    def b_phase(bx_s, y_s, wrT_s, wiT_s, wd_s, wt_s, xre_s, xim_s, ys_s,
                gdf_s, gnf_s, gsf_s, gsi_s, bsem):
        def bcopy(src, dst, i):
            return pltpu.make_async_copy(src, dst, bsem.at[i])
        nch = S // BR
        xc = [bcopy(bx_hbm.at[pl.ds(i * BR, BR), :], bx_s.at[pl.ds(i * BR, BR), :], i)
              for i in range(nch)]
        cc = [bcopy(gdf_hbm, gdf_s, nch), bcopy(gnf_hbm, gnf_s, nch + 1),
              bcopy(wrT_hbm, wrT_s, nch + 2), bcopy(wiT_hbm, wiT_s, nch + 3),
              bcopy(gsf_hbm, gsf_s, nch + 4), bcopy(gsi_hbm, gsi_s, nch + 5)]
        xc[0].start()
        cc[0].start()
        cc[1].start()
        xc[1].start()

        cc[0].wait()
        cc[1].wait()
        xc[0].wait()
        xc[2].start()
        _b_d_forward_vpu(bx_s, y_s, 0, 0, BR)

        for i in range(nch):
            if i + 1 < nch:
                xc[i + 1].wait()
            if i == 0:
                xc[3].start()
            if i == 2:
                cc[2].start()
                cc[3].start()
            for a in range(0, BR, DSUB):
                _b_d_forward_mxu(y_s, i % 2, gdf_s, gnf_s, xre_s, xim_s, i * BR, a, DSUB)
                if i + 1 < nch:
                    for b in range(a, a + DSUB, VSL):
                        _b_d_forward_vpu_slab(bx_s, y_s, (i + 1) % 2, (i + 1) * BR, b)

        cc[2].wait()
        cc[3].wait()
        cc[4].start()
        cc[5].start()
        copy(ac_hbm, ac_s, 1).start()

        def p1(i, c):
            @pl.when(i == DMA_A)
            def _():
                copy(ax_hbm, ax_s, 0).start()
            if P1ORD == 0:
                for v in range(2):
                    _b_prepare_w(wrT_s, wiT_s, wd_s, wt_s, 2 * i + v)
            for v in range(NCT):
                u = i * NCT + v
                _b_s_pass1(xre_s, xim_s, ys_s, u // 8, u % 8)
            if P1ORD == 1:
                for v in range(2):
                    _b_prepare_w(wrT_s, wiT_s, wd_s, wt_s, 2 * i + v)
            return c
        lax.fori_loop(0, 8, p1, 0)
        cc[4].wait()
        cc[5].wait()
        copy(ac_hbm, ac_s, 1).wait()
        for cp in wcopies(0):
            cp.start()

        npi = N1 // P2U

        def p2(kk, c):
            @pl.when(kk == npi - 1)
            def _():
                for v in range(NWO):
                    for cp in wocopies(v):
                        cp.start()
                copy(gdi_hbm, gdi_s, 8).start()
                copy(gni_hbm, gni_s, 9).start()
            _b_s_pass2(ys_s, zs_s, wt_s, gsf_s, gsi_s, [kk * P2U + u for u in range(P2U)])
            return c
        lax.fori_loop(0, N1 // P2U, p2, 0)

    def b_scope():
      pl.run_scoped(
        b_phase,
        pltpu.VMEM((S, DM), BF16), pltpu.VMEM((2, BR // 2, DM), U32),
        pltpu.VMEM((DF, S), BF16), pltpu.VMEM((DF, S), BF16),
        pltpu.VMEM((S // T, 512, T), U32), pltpu.VMEM((NCT, S, T), U32),
        pltpu.VMEM((NCT, S, T), F32), pltpu.VMEM((NCT, S, T), F32),
        pltpu.VMEM((N1, NCT, T, T), BF16),
        pltpu.VMEM((4, 128, 256), U32), pltpu.VMEM((T // 2, T), U32),
        pltpu.VMEM((N1, T // 2, T), U32), pltpu.VMEM((N1, T // 2, T), U32),
        pltpu.SemaphoreType.DMA((S // BR + 6,)),
    )

    def a_outer(ctx_s, wos_s):
        def a_main(wu_s, q_s, k_s, v_s):
            def stage_w(i, chain):
                rows = (DM + 2 * DC) // 8
                step = WSL2 if chain else 128
                for a in range(0, rows, step):
                    r = pl.multiple_of(i * rows + a, step)
                    v = w_st[pl.ds(r, step)]
                    wu_s[pl.ds(pl.multiple_of(4 * r, 4 * step), 4 * step), :] = pltpu.bitcast(
                        v.reshape(step * 8, HD), U32)
                    if chain:
                        w_st[DM + 2 * DC:DM + 2 * DC + 2] = v[0:2]

            def w_rhs(slot, base, kk):
                def blk(m0, hp0):
                    cols = []
                    for hp in (hp0, hp0 + 1):
                        x = wu_s[pl.ds(4 * m0 + hp, kk, stride=4), :]
                        cols.append(pltpu.bitcast(x << 16, F32))
                        cols.append(pltpu.bitcast(x & jnp.uint32(0xFFFF0000), F32))
                    return jnp.concatenate(cols, axis=1)
                b11, b12 = blk(base, 0), blk(base, 2)
                b21, b22 = blk(base + kk, 0), blk(base + kk, 2)
                return [v.astype(BF16) for v in _rhs_ops(b11, b12, b21, b22)]

            def prep_wo(u, chain):
                step = WSL if chain else T
                for a in range(0, T, step):
                    r = pl.multiple_of(u * T + a, step)
                    top = wo_s[pl.ds(r, step), :].astype(F32)
                    bot = wo_s[pl.ds(H * HD // 2 + r, step), :].astype(F32)
                    ops = _rhs_ops(top[:, :512], top[:, 512:], bot[:, :512], bot[:, 512:])
                    for jj, j in enumerate((0, 2, 3, 5, 6)):
                        v = ops[j].astype(BF16)
                        wos_s[jj, pl.ds(r, step), :] = v
                    if chain:
                        wo_s[H * HD:H * HD + 16, 0:HD] = v[0:16, 0:HD]

            copy(ax_hbm, ax_s, 0).wait()
            for cp in wcopies(0):
                cp.wait()

            def prew(i, c):
                stage_w(i, False)
                return c
            lax.fori_loop(0, 8, prew, 0)

            def lhs7(src, r):
                kk = src.shape[1] // 2
                top, bot = pl.ds(r, PR), pl.ds(HS + r, PR)
                a11, a12, a21, a22 = src[top, :kk], src[top, kk:], src[bot, :kk], src[bot, kk:]
                sm = [v.astype(BF16) for v in _lhs_sums(*[v.astype(F32) for v in (a11, a12, a21, a22)])]
                return (sm[0], sm[1], a11, a22, sm[2], sm[3], sm[4])

            def group(g, c):
                slot = 0
                gn = jnp.minimum(g + 1, NG - 1)
                for cp in wcopies(gn):
                    cp.start()

                def chunk(i, cc):
                    r = pl.multiple_of(i * PR, PR)
                    top, bot = pl.ds(r, PR), pl.ds(HS + r, PR)
                    for cp in wocopies(g * 4 + i):
                        cp.wait()

                    def put(dst, cs, scale=None):
                        top2 = pl.ds(pl.multiple_of(i * (PR // 2), PR // 2), PR // 2)
                        bot2 = pl.ds(pl.multiple_of(HS // 2 + i * (PR // 2), PR // 2), PR // 2)
                        for cb, rows, h0 in zip(cs, (top2, top2, bot2, bot2), (0, 4, 0, 4)):
                            if scale is not None:
                                cb = cb * scale
                            cb = _pk(cb)
                            for hh in range(4):
                                dst[h0 + hh, rows, :] = cb[:, hh * HD:(hh + 1) * HD]
                    cl = lhs7(ac_s, r)
                    put(k_s, _strassen(cl, w_rhs(slot, DM, DC // 2)))
                    put(v_s, _strassen(cl, w_rhs(slot, DM + DC, DC // 2)))
                    put(q_s, _strassen(lhs7(ax_s, r), w_rhs(slot, 0, DM // 2)), Q_SCALE)
                    if WORD < 9: prep_wo(g * 4 + i, True)
                    return cc
                lax.fori_loop(0, HS // PR, chunk, 0)

                for cp in wcopies(gn):
                    cp.wait()

                def head(hh, cc):
                    h = hh * AUN
                    _attn_heads(q_s, k_s, v_s, ctx_s, h, g * 8 + h)
                    for u in range(AUN):
                        stage_w(h + u, True)
                    return cc
                lax.fori_loop(0, 8 // AUN, head, 0)
                return c
            lax.fori_loop(0, NG, group, 0)

        b_scope()
        pl.run_scoped(a_main, pltpu.VMEM((4 * (DM + 2 * DC), HD), U32),
                      *[pltpu.VMEM((8, S // 2, HD), U32)] * 3)

        def a_out(oa_s, yb_s, xre_s, xim_s, osem):
            nch = HS // OR

            def ocopies(i):
                r = pl.multiple_of(i * OR, OR)
                r2 = pl.multiple_of(HS + i * OR, OR)
                return (pltpu.make_async_copy(oa_s.at[pl.ds(r, OR), :],
                                              out_hbm.at[pl.ds(r, OR), pl.ds(0, DM)], osem.at[2 * i]),
                        pltpu.make_async_copy(oa_s.at[pl.ds(r2, OR), :],
                                              out_hbm.at[pl.ds(r2, OR), pl.ds(0, DM)], osem.at[2 * i + 1]))

            def ycopy(i):
                r = pl.multiple_of(i * BR, BR)
                return pltpu.make_async_copy(yb_s.at[pl.ds(r, BR), :],
                                             out_hbm.at[pl.ds(r, BR), pl.ds(DM, DM)], osem.at[2 * nch + i])

            def blk(rows, h0):
                return [_ld(ctx_s, h0 + h, rows) for h in range(H // 2)]

            def ochunk(i, c):
                r = pl.multiple_of(i * OR, OR)
                top, bot = pl.ds(r, OR), pl.ds(HS + r, OR)
                cat = lambda xs: jnp.concatenate(xs, axis=1)
                hk = H * HD // 2
                top2 = pl.ds(pl.multiple_of(i * (OR // 2), OR // 2), OR // 2)
                bot2 = pl.ds(pl.multiple_of(HS // 2 + i * (OR // 2), OR // 2), OR // 2)
                a11, a22 = cat(blk(top2, 0)), cat(blk(bot2, 16))
                m3 = _dot(a11, wos_s[1])
                m4 = _dot(a22, wos_s[2])
                a12, a21 = cat(blk(top2, 16)), cat(blk(bot2, 0))
                sums = [v.astype(BF16) for v in
                        _lhs_sums(*[v.astype(F32) for v in (a11, a12, a21, a22)])]
                m1 = _dot(sums[0], wos_s[0])
                m2 = _dot(sums[1], wo_s[0:hk, 0:512])
                m5 = _dot(sums[2], wo_s[hk:2 * hk, 512:1024])
                m6 = _dot(sums[3], wos_s[3])
                m7 = _dot(sums[4], wos_s[4])
                cs = (((m1 + m4) - m5) + m7, m3 + m5, m2 + m4, ((m1 - m2) + m3) + m6)
                for cb, rows, c0 in zip(cs, (top, top, bot, bot), (0, 512, 0, 512)):
                    oa_s[rows, c0:c0 + 512] = cb.astype(BF16)
                for v in range(NCT * 8 // nch):
                    u = i * (NCT * 8 // nch) + v
                    _b_s_pass3(zs_s, xre_s, xim_s, u // 8, u % 8, True)
                for cp in ocopies(i):
                    cp.start()
                return c
            lax.fori_loop(0, nch, ochunk, 0)

            copy(gdi_hbm, gdi_s, 8).wait()
            copy(gni_hbm, gni_s, 9).wait()

            def dinv(i, c):
                _b_d_inverse(xre_s, xim_s, gdi_s, gni_s, yb_s, pl.multiple_of(i * BR, BR), BR)
                ycopy(i).start()
                return c
            lax.fori_loop(0, S // BR, dinv, 0)
            for i in range(nch):
                for cp in ocopies(i):
                    cp.wait()
            for i in range(S // BR):
                ycopy(i).wait()

        pl.run_scoped(a_out, pltpu.VMEM((S, DM), BF16), pltpu.VMEM((S, DM), BF16),
                      pltpu.VMEM((NCT, S, T), F32), pltpu.VMEM((NCT, S, T), F32),
                      pltpu.SemaphoreType.DMA((2 * (HS // OR) + S // BR,)))

    pl.run_scoped(a_outer, pltpu.VMEM((H, S // 2, HD), U32), pltpu.VMEM((5, H * HD // 2, 512), BF16))


@jax.jit
def pallas_concat_heads__compressed_kv_cla__spectral_gfnet__prompt_kernel(
    A_x, A_c_kv, A_w_q, A_w_uk, A_w_uv, A_w_o, B_x, B_w_r, B_w_i,
):
    hbm = pl.BlockSpec(memory_space=pl.ANY)
    out = pl.pallas_call(
        _kernel,
        in_specs=[hbm] * 15,
        out_specs=hbm,
        out_shape=jax.ShapeDtypeStruct((S, 2 * DM), BF16),
        scratch_shapes=[
            pltpu.VMEM((S, DM), BF16), pltpu.VMEM((S, DC), BF16),
            pltpu.VMEM((DM + 2 * DC + 2, 8, HD), BF16),
            pltpu.VMEM((H * HD + 16, DM), BF16),
            pltpu.VMEM((N1 + 1, NCT, T, T), BF16),
            pltpu.VMEM((4, 128, 256), U32), pltpu.VMEM((T // 2, T), U32),
            pltpu.SemaphoreType.DMA((10,)), pltpu.SemaphoreType.DMA((2 * NWO,)),
        ],
        compiler_params=pltpu.CompilerParams(vmem_limit_bytes=120 * 1024 * 1024),
    )(A_x.reshape(S, DM), A_c_kv.reshape(S, DC), A_w_q, A_w_uk, A_w_uv,
      A_w_o.reshape(H * HD, DM), B_x.reshape(S, DM), B_w_r.T, B_w_i.T, *_CONSTS)
    return out.reshape(1, S, 2 * DM)
```

```python
import functools
import math

import jax
import jax.numpy as jnp
import numpy as np
from jax import lax
from jax.experimental import pallas as pl
from jax.experimental.pallas import tpu as pltpu

S = 2048
DM = 1024
DC = 512
H = 32
HD = 128
T = 128
NG = 4
DF = DM // 2 + 1
NCT = 5
N1, N2 = 32, 64

F32, BF16, U32 = jnp.float32, jnp.bfloat16, jnp.uint32
LOG2E = math.log2(math.e)
Q_SCALE = float(HD ** -0.5 * LOG2E)
MASK_VAL = float(-1e9 * LOG2E)
CLASS_PAIRS = ((0, 4), (1, 7), (2, 6), (3, 5))


def _make_constants():
    b = np.arange(128)[:, None].astype(np.float64)
    m = np.arange(64)[None, :].astype(np.float64)

    def cs(r):
        th = 2.0 * np.pi * b * (r + 8.0 * m) / DM
        return np.cos(th), np.sin(th)

    gdf = np.zeros((4, 256, 256))
    c0, s0 = cs(0)
    c4, s4 = cs(4)
    gdf[0, :128, 0:64], gdf[0, :128, 128:192] = c0, -s0
    gdf[0, 128:, 64:128], gdf[0, 128:, 192:256] = c4, -s4
    for p in (1, 2, 3):
        r, r2 = CLASS_PAIRS[p]
        c, s = cs(r)
        c2, s2 = cs(r2)
        gdf[p, :128, 0:64], gdf[p, 128:, 0:64] = c, s
        gdf[p, :128, 64:128], gdf[p, 128:, 64:128] = c2, -s2
        gdf[p, :128, 128:192], gdf[p, 128:, 128:192] = -s, c
        gdf[p, :128, 192:256], gdf[p, 128:, 192:256] = -s2, -c2
    alt = (-1.0) ** np.arange(128)
    gnf = np.zeros((128, 128))
    gnf[:, 0] = alt

    sc = 1.0 / (S * DM)
    gdi = np.zeros((4, 256, 256))
    w0 = np.full((64, 1), 2.0)
    w0[0] = 1.0
    gdi[0, 0:64, 0:128] = (c0.T * w0) * sc
    gdi[0, 128:192, 0:128] = (-s0.T * w0) * sc
    gdi[0, 128, :] = 0.0
    gdi[0, 64:128, 128:256] = 2.0 * c4.T * sc
    gdi[0, 192:256, 128:256] = -2.0 * s4.T * sc
    for p in (1, 2, 3):
        r, r2 = CLASS_PAIRS[p]
        c, s = cs(r)
        c2, s2 = cs(r2)
        f = 2.0 * sc
        gdi[p, 0:64, 0:128], gdi[p, 128:192, 0:128] = f * c.T, -f * s.T
        gdi[p, 64:128, 0:128], gdi[p, 192:256, 0:128] = f * c2.T, -f * s2.T
        gdi[p, 0:64, 128:256], gdi[p, 128:192, 128:256] = f * s.T, f * c.T
        gdi[p, 64:128, 128:256], gdi[p, 192:256, 128:256] = -f * s2.T, -f * c2.T
    gni = np.zeros((128, 128))
    gni[0, :] = alt * sc

    n2 = np.arange(N2)
    perm = np.concatenate([np.concatenate([8 * j + np.arange(8), 64 + 8 * j + np.arange(8)])
                           for j in range(8)])
    gsf = np.zeros((N1, 128, 128))
    gsi = np.zeros((N1, 128, 128))
    for k1 in range(N1):
        k = k1 + N1 * n2
        g = np.exp(-2j * np.pi * np.outer(k, n2) / S)
        ghat = np.block([[g.real, -g.imag], [g.imag, g.real]])
        gsf[k1] = ghat[perm][:, perm]
        gsi[k1] = ghat.T[perm][:, perm]
    def words(a):
        u = np.asarray(a, dtype=np.float32).astype(jnp.bfloat16).view(np.uint16).astype(np.uint32)
        return np.ascontiguousarray(u[..., 0::2, :] | (u[..., 1::2, :] << 16))
    return tuple(words(a) for a in (gdf, gnf, gdi, gni, gsf, gsi))


_CONSTS = _make_constants()


def _dot(a, b):
    return jnp.dot(a, b, preferred_element_type=F32)


def _dot_nt(a, b):
    return lax.dot_general(a, b, (((1,), (1,)), ((), ())), preferred_element_type=F32)


def _ld(ref, *idx):
    return pltpu.bitcast(ref[idx], BF16)


def _pk(v):
    return pltpu.bitcast(v.astype(BF16), U32)


def _rows(r0, n):
    return pl.ds(r0 // 2, n // 2)


def _cmul_const(x, e, n, sign):
    re, im = x
    e %= n
    if e == 0:
        return re, im
    if 8 * e % n == 0:
        o = 8 * e // n
        if sign < 0:
            o = (8 - o) % 8
        h = math.sqrt(0.5)
        if o == 2:
            return -im, re
        if o == 4:
            return -re, -im
        if o == 6:
            return im, -re
        if o == 1:
            return (re - im) * h, (re + im) * h
        if o == 3:
            return (re + im) * (-h), (re - im) * h
        if o == 5:
            return (im - re) * h, (re + im) * (-h)
        if o == 7:
            return (re + im) * h, (im - re) * h
    th = sign * 2.0 * math.pi * e / n
    c, s = math.cos(th), math.sin(th)
    return re * c - im * s, re * s + im * c


def _cadd(a, b):
    return a[0] + b[0], a[1] + b[1]


def _csub(a, b):
    return a[0] - b[0], a[1] - b[1]


def _fft(xs, sign):
    n = len(xs)
    if n == 1:
        return xs
    if n == 2:
        return [_cadd(xs[0], xs[1]), _csub(xs[0], xs[1])]
    u = _fft(xs[0::2], sign)
    z1 = _fft(xs[1::4], sign)
    z3 = _fft(xs[3::4], sign)
    out = [None] * n
    q = n // 4
    for k in range(q):
        a = _cmul_const(z1[k], k, n, sign)
        b = _cmul_const(z3[k], 3 * k, n, sign)
        sm, df = _cadd(a, b), _csub(a, b)
        out[k] = _cadd(u[k], sm)
        out[k + 2 * q] = _csub(u[k], sm)
        if sign < 0:
            out[k + q] = (u[k + q][0] + df[1], u[k + q][1] - df[0])
            out[k + 3 * q] = (u[k + q][0] - df[1], u[k + q][1] + df[0])
        else:
            out[k + q] = (u[k + q][0] - df[1], u[k + q][1] + df[0])
            out[k + 3 * q] = (u[k + q][0] + df[1], u[k + q][1] - df[0])
    return out


def _b_words(a, b):
    return (pltpu.bitcast(a.astype(F32), U32) >> 16) | (
        pltpu.bitcast(b.astype(F32), U32) & jnp.uint32(0xFFFF0000))


def _b_prepare_w_words(wrT_s, wiT_s, wd_s, t):
    cols = pl.ds(pl.multiple_of(t * T, T), T)
    for a in range(0, 512, 64):
        wd_s[t, a:a + 64, :] = _b_words(wrT_s[a:a + 64, cols], wiT_s[a:a + 64, cols])


def _b_prepare_w_order(wrT_s, wiT_s, wd_s, wt_s, t):
    rows = pl.ds(pl.multiple_of(t * T, T), T)
    for p, (r, r2) in enumerate(CLASS_PAIRS):
        a = wd_s[t, pl.ds(r, 64, stride=8), :]
        b = wd_s[t, pl.ds(r2, 64, stride=8), :]
        wt_s[p, rows, :] = jnp.concatenate([a, b], axis=0).T
    ny = _b_words(wrT_s[512:513, rows], wiT_s[512:513, rows])
    row = lax.broadcasted_iota(jnp.int32, (T, T), 0)
    wt_s[4, rows, :] = jnp.where(row == 0, jnp.broadcast_to(ny, (T, T)), jnp.uint32(0)).T


def _b_d_forward_vpu(xb_s, y_s, slot, r0, rows):
    for a in range(0, rows, VSL):
        _b_d_forward_vpu_slab(xb_s, y_s, slot, r0, a)


def _b_d_forward_vpu_slab(xb_s, y_s, slot, r0, a):
    sl = pl.ds(r0 + a, VSL)
    x = [xb_s[sl, a * T:(a + 1) * T].astype(F32) for a in range(8)]
    s04, t = x[0] + x[4], x[0] - x[4]
    s26, u = x[2] + x[6], x[2] - x[6]
    s15, v = x[1] + x[5], x[1] - x[5]
    s37, w = x[3] + x[7], x[3] - x[7]
    e, f = s04 + s26, s04 - s26
    g, hh = s15 + s37, s15 - s37
    k = math.sqrt(0.5)
    al, be = (v - w) * k, (v + w) * k
    ys = ((e + g, e - g),
          (t + al, -(u + be)),
          (f, -hh),
          (t - al, u - be))
    for p in range(4):
        y_s[slot, a // 2:(a + VSL) // 2, 2 * p * T:(2 * p + 2) * T] = _pk(jnp.concatenate(
            [ys[p][0], ys[p][1]], axis=1))


def _b_d_forward_mxu(y_s, slot, gdf_s, gnf_s, xre_s, xim_s, r0, a, rows):
    sl = pl.ds(r0 + a, rows)
    for p in range(4):
        o = _dot(_ld(y_s, slot, slice(a // 2, (a + rows) // 2), slice(2 * p * T, (2 * p + 2) * T)), _ld(gdf_s, p))
        xre_s[p, sl, :] = o[:, :T]
        xim_s[p, sl, :] = o[:, T:]
    xre_s[4, sl, :] = _dot(_ld(y_s, slot, slice(a // 2, (a + rows) // 2), slice(0, T)),
                           pltpu.bitcast(gnf_s[...], BF16))
    xim_s[4, sl, :] = jnp.zeros((rows, T), F32)


def _fft32(load, emit, sign):
    half = N1 // 2
    for par in range(2):
        xs = []
        for n in range(half):
            a, b = load(n), load(n + half)
            xs.append(_cadd(a, b) if par == 0 else _cmul_const(_csub(a, b), n, N1, sign))
        out = _fft(xs, sign)
        for q in range(half):
            emit(2 * q + par, out[q])


def _b_s_pass1(xre_s, xim_s, ys_s, c, j):
    off = pl.multiple_of(j * 8, 8)

    def load(n1):
        rows = pl.ds(N2 * n1 + off, 8)
        return xre_s[c, rows, :], xim_s[c, rows, :]

    def emit(k1, v):
        ys_s[k1, c, pl.ds(pl.multiple_of(j * 16, 16), 16), :] = jnp.concatenate(v, axis=0).astype(BF16)
    _fft32(load, emit, -1)


def _b_s_pass2_fwd(ys_s, gsf_s, k1):
    rhs = jnp.concatenate([ys_s[k1, c] for c in range(NCT)], axis=1)
    return _dot(_ld(gsf_s, k1), rhs)


def _b_s_pass2_inv(vv, zs_s, wt_s, gsi_s, k1):
    outs = []
    for c in range(NCT):
        wd = wt_s[c, pl.ds(k1, N2, stride=N1), :]
        wr = pltpu.bitcast(wd << 16, F32)
        wi = pltpu.bitcast(wd & jnp.uint32(0xFFFF0000), F32)
        pcs = []
        for j in range(8):
            vr = vv[16 * j:16 * j + 8, c * T:(c + 1) * T]
            vi = vv[16 * j + 8:16 * j + 16, c * T:(c + 1) * T]
            a, b = wr[8 * j:8 * j + 8], wi[8 * j:8 * j + 8]
            pcs.append(vr * a - vi * b)
            pcs.append(vr * b + vi * a)
        outs.append(jnp.concatenate(pcs, axis=0).astype(BF16))
    ginv = _ld(gsi_s, k1)
    for c in range(NCT):
        zs_s[k1, c] = _dot(ginv, outs[c]).astype(BF16)


def _b_s_pass2(ys_s, zs_s, wt_s, gsf_s, gsi_s, k1s):
    pend = []
    for a in range(len(k1s) + P2D):
        if a < len(k1s):
            pend.append(_b_s_pass2_fwd(ys_s, gsf_s, k1s[a]))
        if a >= P2D:
            _b_s_pass2_inv(pend.pop(0), zs_s, wt_s, gsi_s, k1s[a - P2D])


def _b_s_pass3(zs_s, xre_s, xim_s, c, j, chain):
    off = pl.multiple_of(j * 8, 8)

    def load(k1):
        z = zs_s[k1, c, pl.ds(pl.multiple_of(j * 16, 16), 16), :].astype(F32)
        return z[0:8], z[8:16]

    def emit(n1, v):
        rows = pl.ds(N2 * n1 + off, 8)
        xre_s[c, rows, :] = v[0]
        xim_s[c, rows, :] = v[1]
        if chain and n1 >= N1 - 2:
            zs_s[N1, 0, 0:16, :] = jnp.concatenate(v, axis=0).astype(BF16)
    _fft32(load, emit, +1)


def _b_d_inverse(xre_s, xim_s, gdi_s, gni_s, yb_s, r0, rows):
    sl = pl.ds(r0, rows)
    us = []
    for p in range(4):
        lhs = jnp.concatenate([xre_s[p, sl, :], xim_s[p, sl, :]], axis=1).astype(BF16)
        o = _dot(lhs, _ld(gdi_s, p))
        us.append((o[:, :T], o[:, T:]))
    u0 = us[0][0] + _dot(xre_s[4, sl, :].astype(BF16), pltpu.bitcast(gni_s[...], BF16))
    u4 = us[0][1]
    (u1r, u1i), (u2r, u2i), (u3r, u3i) = us[1], us[2], us[3]
    e0, e1 = u0 + u4, u0 - u4
    ev = (e0 + u2r, e1 - u2i, e0 - u2r, e1 + u2i)
    pq, qq = u1r - u3r, u1i + u3i
    k = math.sqrt(0.5)
    od = (u1r + u3r, (pq - qq) * k, u3i - u1i, (pq + qq) * (-k))
    for a in range(4):
        yb_s[sl, a * T:(a + 1) * T] = (ev[a] + od[a]).astype(BF16)
        yb_s[sl, (a + 4) * T:(a + 5) * T] = (ev[a] - od[a]).astype(BF16)


VSL = 16
BQ = 128
ADEPTH = 2
ACK = 128
AORD = 2
AUN = 2


def _attn_order(h0):
    n = S // BQ
    if AORD == 0:
        return [(h0 + u, i) for u in range(AUN) for i in range(n - 1, -1, -1)]
    if AORD == 1:
        return [p for i in range(n) for p in ((h0, n - 1 - i), (h0 + 1, i))]
    if AORD == 2:
        o = []
        lo, hi = 0, n - 1
        while lo <= hi:
            o.append(hi)
            hi -= 1
            if lo <= hi:
                o.append(lo)
                lo += 1
        return [(h0 + u, i) for u in range(AUN) for i in o]


def _attn_heads(q_s, k_s, v_s, o_s, h0, ho):
    nt = BQ // T
    row = lax.broadcasted_iota(jnp.int32, (T, T), 0)
    col = lax.broadcasted_iota(jnp.int32, (T, T), 1)
    causal = col <= row

    def scores(h, i):
        r0 = i * BQ
        nfull = r0 // T + 1
        tiles = {}
        s = _dot_nt(_ld(q_s, h, _rows(r0, BQ)), _ld(k_s, h, _rows(0, nfull * T)))
        for t in range(nt):
            for j in range(nfull):
                tiles[t, j] = s[t * T:(t + 1) * T, j * T:(j + 1) * T]
        for t in range(1, nt):
            j = nfull - 1 + t
            st = _dot_nt(_ld(q_s, h, _rows(r0 + t * T, BQ - t * T)), _ld(k_s, h, _rows(j * T, T)))
            for u in range(t, nt):
                tiles[u, j] = st[(u - t) * T:(u - t + 1) * T]
        for t in range(nt):
            jd = nfull - 1 + t
            tiles[t, jd] = jnp.where(causal, tiles[t, jd], MASK_VAL)
        return tiles

    def softmax_pv(h, i, tiles):
        r0 = i * BQ
        nfull = r0 // T + 1
        for t in range(nt):
            nk = nfull + t
            mx = tiles[t, 0]
            for j in range(1, nk):
                mx = jnp.maximum(mx, tiles[t, j])
            m = jnp.max(mx, axis=1, keepdims=True)
            lacc = o = None
            cj = ACK // T
            for j0 in range(0, nk, cj):
                ps = []
                for j in range(j0, min(nk, j0 + cj)):
                    p = jnp.exp2(tiles[t, j] - m)
                    lacc = p if lacc is None else lacc + p
                    ps.append(p)
                pc = jnp.concatenate(ps, axis=1) if len(ps) > 1 else ps[0]
                oo = _dot(pc.astype(BF16), _ld(v_s, h, _rows(j0 * T, len(ps) * T)))
                o = oo if o is None else o + oo
            l = jnp.sum(lacc, axis=1, keepdims=True)
            o_s[h - h0 + ho, _rows(r0 + t * T, T)] = _pk(o * pl.reciprocal(l, approx=True))

    order = _attn_order(h0)
    pend = []
    for a in range(len(order) + ADEPTH):
        if a < len(order):
            pend.append(scores(*order[a]))
        if a >= ADEPTH:
            softmax_pv(*order[a - ADEPTH], pend.pop(0))


HS = S // 2


def _lhs_sums(a11, a12, a21, a22):
    return (a11 + a22, a21 + a22, a11 + a12, a21 - a11, a12 - a22)


def _rhs_ops(b11, b12, b21, b22):
    return (b11 + b22, b11, b12 - b22, b21 - b11, b22, b11 + b12, b21 + b22)


def _strassen(lhs, rhs):
    m3, m4 = _dot(lhs[2], rhs[2]), _dot(lhs[3], rhs[3])
    m1, m2, m5, m6, m7 = [_dot(lhs[j], rhs[j]) for j in (0, 1, 4, 5, 6)]
    return (((m1 + m4) - m5) + m7, m3 + m5, m2 + m4, ((m1 - m2) + m3) + m6)


PR = 256
OR = 128
BR = 512
DSUB = 64
P2D = 1
P2U = 8
WSL = 16
WSL2 = 32
OCH = 1
AREP = 1
DMA_A = 4
DMA_B = 32
DSUB2 = 128
WPIN = 0
PORD = 3
WORD = 3
NWO = 16


def _kernel(ax_hbm, ac_hbm, wq_hbm, wuk_hbm, wuv_hbm, wo_hbm, bx_hbm, wrT_hbm, wiT_hbm,
            gdf_hbm, gnf_hbm, gdi_hbm, gni_hbm, gsf_hbm, gsi_hbm,
            out_hbm,
            ax_s, ac_s, w_st, wo_s, zs_s, gdi_s, gni_s, sems, wosem):
    def copy(src, dst, i):
        return pltpu.make_async_copy(src, dst, sems.at[i])

    def wcopies(g):
        hs = pl.ds(pl.multiple_of(g * 8, 8), 8)
        return (copy(wq_hbm.at[:, hs, :], w_st.at[pl.ds(0, DM)], 2),
                copy(wuk_hbm.at[:, hs, :], w_st.at[pl.ds(DM, DC)], 3),
                copy(wuv_hbm.at[:, hs, :], w_st.at[pl.ds(DM + DC, DC)], 4))

    def wocopies(u):
        r = pl.multiple_of(u * T, T)
        r2 = pl.multiple_of(H * HD // 2 + u * T, T)
        return (pltpu.make_async_copy(wo_hbm.at[pl.ds(r, T), :], wo_s.at[pl.ds(r, T), :], wosem.at[2 * u]),
                pltpu.make_async_copy(wo_hbm.at[pl.ds(r2, T), :], wo_s.at[pl.ds(r2, T), :], wosem.at[2 * u + 1]))

    def b_phase(bx_s, y_s, wrT_s, wiT_s, wd_s, wt_s, xre_s, xim_s, ys_s,
                gdf_s, gnf_s, gsf_s, gsi_s, bsem):
        def bcopy(src, dst, i):
            return pltpu.make_async_copy(src, dst, bsem.at[i])
        nch = S // BR
        xc = [bcopy(bx_hbm.at[pl.ds(i * BR, BR), :], bx_s.at[pl.ds(i * BR, BR), :], i)
              for i in range(nch)]
        cc = [bcopy(gdf_hbm, gdf_s, nch), bcopy(gnf_hbm, gnf_s, nch + 1),
              bcopy(wrT_hbm, wrT_s, nch + 2), bcopy(wiT_hbm, wiT_s, nch + 3),
              bcopy(gsf_hbm, gsf_s, nch + 4), bcopy(gsi_hbm, gsi_s, nch + 5)]
        xc[0].start()
        cc[0].start()
        cc[1].start()
        xc[1].start()

        cc[0].wait()
        cc[1].wait()
        xc[0].wait()
        xc[2].start()
        _b_d_forward_vpu(bx_s, y_s, 0, 0, BR)

        for i in range(nch):
            if i + 1 < nch:
                xc[i + 1].wait()
            if i == 0:
                xc[3].start()
            if i == 2:
                cc[2].start()
                cc[3].start()
            for a in range(0, BR, DSUB):
                _b_d_forward_mxu(y_s, i % 2, gdf_s, gnf_s, xre_s, xim_s, i * BR, a, DSUB)
                if i + 1 < nch:
                    for b in range(a, a + DSUB, VSL):
                        _b_d_forward_vpu_slab(bx_s, y_s, (i + 1) % 2, (i + 1) * BR, b)

        cc[2].wait()
        cc[3].wait()
        cc[4].start()
        cc[5].start()
        copy(ac_hbm, ac_s, 1).start()

        def p1(i, c):
            @pl.when(i == DMA_A)
            def _():
                copy(ax_hbm, ax_s, 0).start()
            for v in range(2):
                _b_prepare_w_order(wrT_s, wiT_s, wd_s, wt_s, 2 * i + v)
            for v in range(NCT):
                u = i * NCT + v
                _b_s_pass1(xre_s, xim_s, ys_s, u // 8, u % 8)
            for v in range(2):
                _b_prepare_w_words(wrT_s, wiT_s, wd_s, jnp.minimum(2 * i + 2 + v, S // T - 1))
            return c
        for v in range(2):
            _b_prepare_w_words(wrT_s, wiT_s, wd_s, v)
        lax.fori_loop(0, 8, p1, 0)
        cc[4].wait()
        cc[5].wait()
        copy(ac_hbm, ac_s, 1).wait()
        for cp in wcopies(0):
            cp.start()

        npi = N1 // P2U

        def p2(kk, c):
            @pl.when(kk == npi - 1)
            def _():
                for v in range(NWO):
                    for cp in wocopies(v):
                        cp.start()
                copy(gdi_hbm, gdi_s, 8).start()
                copy(gni_hbm, gni_s, 9).start()
            _b_s_pass2(ys_s, zs_s, wt_s, gsf_s, gsi_s, [kk * P2U + u for u in range(P2U)])
            return c
        lax.fori_loop(0, N1 // P2U, p2, 0)

    def b_scope():
      pl.run_scoped(
        b_phase,
        pltpu.VMEM((S, DM), BF16), pltpu.VMEM((2, BR // 2, DM), U32),
        pltpu.VMEM((DF, S), BF16), pltpu.VMEM((DF, S), BF16),
        pltpu.VMEM((S // T, 512, T), U32), pltpu.VMEM((NCT, S, T), U32),
        pltpu.VMEM((NCT, S, T), F32), pltpu.VMEM((NCT, S, T), F32),
        pltpu.VMEM((N1, NCT, T, T), BF16),
        pltpu.VMEM((4, 128, 256), U32), pltpu.VMEM((T // 2, T), U32),
        pltpu.VMEM((N1, T // 2, T), U32), pltpu.VMEM((N1, T // 2, T), U32),
        pltpu.SemaphoreType.DMA((S // BR + 6,)),
    )

    def a_outer(ctx_s, wos_s):
        def a_main(wu_s, q_s, k_s, v_s):
            def stage_w(i, chain):
                rows = (DM + 2 * DC) // 8
                step = WSL2 if chain else 128
                for a in range(0, rows, step):
                    r = pl.multiple_of(i * rows + a, step)
                    v = w_st[pl.ds(r, step)]
                    wu_s[pl.ds(pl.multiple_of(4 * r, 4 * step), 4 * step), :] = pltpu.bitcast(
                        v.reshape(step * 8, HD), U32)
                    if chain:
                        w_st[DM + 2 * DC:DM + 2 * DC + 2] = v[0:2]

            def w_rhs(slot, base, kk):
                def blk(m0, hp0):
                    cols = []
                    for hp in (hp0, hp0 + 1):
                        x = wu_s[pl.ds(4 * m0 + hp, kk, stride=4), :]
                        cols.append(pltpu.bitcast(x << 16, F32))
                        cols.append(pltpu.bitcast(x & jnp.uint32(0xFFFF0000), F32))
                    return jnp.concatenate(cols, axis=1)
                b11, b12 = blk(base, 0), blk(base, 2)
                b21, b22 = blk(base + kk, 0), blk(base + kk, 2)
                return [v.astype(BF16) for v in _rhs_ops(b11, b12, b21, b22)]

            def prep_wo(u, chain):
                step = WSL if chain else T
                for a in range(0, T, step):
                    r = pl.multiple_of(u * T + a, step)
                    top = wo_s[pl.ds(r, step), :].astype(F32)
                    bot = wo_s[pl.ds(H * HD // 2 + r, step), :].astype(F32)
                    ops = _rhs_ops(top[:, :512], top[:, 512:], bot[:, :512], bot[:, 512:])
                    r2 = pl.multiple_of(u * (T // 2) + a // 2, step // 2)
                    for j in range(7):
                        v = ops[j].astype(BF16)
                        wos_s[j, pl.ds(r2, step // 2), :] = pltpu.bitcast(v, U32)
                    if chain:
                        wo_s[H * HD:H * HD + 16, 0:HD] = v[0:16, 0:HD]

            copy(ax_hbm, ax_s, 0).wait()
            for cp in wcopies(0):
                cp.wait()

            def prew(i, c):
                stage_w(i, False)
                return c
            lax.fori_loop(0, 8, prew, 0)

            def lhs7(src, r):
                kk = src.shape[1] // 2
                top, bot = pl.ds(r, PR), pl.ds(HS + r, PR)
                a11, a12, a21, a22 = src[top, :kk], src[top, kk:], src[bot, :kk], src[bot, kk:]
                sm = [v.astype(BF16) for v in _lhs_sums(*[v.astype(F32) for v in (a11, a12, a21, a22)])]
                return (sm[0], sm[1], a11, a22, sm[2], sm[3], sm[4])

            def group(g, c):
                slot = 0
                gn = jnp.minimum(g + 1, NG - 1)
                for cp in wcopies(gn):
                    cp.start()

                def chunk(i, cc):
                    r = pl.multiple_of(i * PR, PR)
                    top, bot = pl.ds(r, PR), pl.ds(HS + r, PR)
                    for cp in wocopies(g * 4 + i):
                        cp.wait()

                    def put(dst, cs, scale=None):
                        top2 = pl.ds(pl.multiple_of(i * (PR // 2), PR // 2), PR // 2)
                        bot2 = pl.ds(pl.multiple_of(HS // 2 + i * (PR // 2), PR // 2), PR // 2)
                        for cb, rows, h0 in zip(cs, (top2, top2, bot2, bot2), (0, 4, 0, 4)):
                            if scale is not None:
                                cb = cb * scale
                            cb = _pk(cb)
                            for hh in range(4):
                                dst[h0 + hh, rows, :] = cb[:, hh * HD:(hh + 1) * HD]
                    cl = lhs7(ac_s, r)
                    kcs = _strassen(cl, w_rhs(slot, DM, DC // 2))
                    put(k_s, kcs)
                    if WPIN == 1:
                        wo_s[H * HD:H * HD + 16, 0:HD] = kcs[1][0:16, 0:HD].astype(BF16)
                        prep_wo(g * 4 + i, True)
                    put(v_s, _strassen(cl, w_rhs(slot, DM + DC, DC // 2)))
                    put(q_s, _strassen(lhs7(ax_s, r), w_rhs(slot, 0, DM // 2)), Q_SCALE)
                    if WPIN == 0: prep_wo(g * 4 + i, True)
                    return cc
                lax.fori_loop(0, HS // PR, chunk, 0)

                for cp in wcopies(gn):
                    cp.wait()

                def head(hh, cc):
                    h = hh * AUN
                    _attn_heads(q_s, k_s, v_s, ctx_s, h, g * 8 + h)
                    for u in range(AUN):
                        stage_w(h + u, True)
                    return cc
                lax.fori_loop(0, 8 // AUN, head, 0)
                return c
            lax.fori_loop(0, NG, group, 0)

        b_scope()
        pl.run_scoped(a_main, pltpu.VMEM((4 * (DM + 2 * DC), HD), U32),
                      *[pltpu.VMEM((8, S // 2, HD), U32)] * 3)

        def a_out(oa_s, yb_s, xre_s, xim_s, osem):
            nch = HS // OR

            def ocopies(i):
                r = pl.multiple_of(i * OR, OR)
                r2 = pl.multiple_of(HS + i * OR, OR)
                return (pltpu.make_async_copy(oa_s.at[pl.ds(r, OR), :],
                                              out_hbm.at[pl.ds(r, OR), pl.ds(0, DM)], osem.at[2 * i]),
                        pltpu.make_async_copy(oa_s.at[pl.ds(r2, OR), :],
                                              out_hbm.at[pl.ds(r2, OR), pl.ds(0, DM)], osem.at[2 * i + 1]))

            def ycopy(i):
                r = pl.multiple_of(i * DSUB2, DSUB2)
                return pltpu.make_async_copy(yb_s.at[pl.ds(r, DSUB2), :],
                                             out_hbm.at[pl.ds(r, DSUB2), pl.ds(DM, DM)], osem.at[16 + i])

            def blk(rows, h0):
                return [_ld(ctx_s, h0 + h, rows) for h in range(H // 2)]

            def ochunk(i, c):
                r = pl.multiple_of(i * OR, OR)
                top, bot = pl.ds(r, OR), pl.ds(HS + r, OR)
                cat = lambda xs: jnp.concatenate(xs, axis=1)
                hk = H * HD // 2
                top2 = pl.ds(pl.multiple_of(i * (OR // 2), OR // 2), OR // 2)
                bot2 = pl.ds(pl.multiple_of(HS // 2 + i * (OR // 2), OR // 2), OR // 2)
                a11, a22 = cat(blk(top2, 0)), cat(blk(bot2, 16))
                m3 = _dot(a11, _ld(wos_s, 2))
                m4 = _dot(a22, _ld(wos_s, 3))
                a12, a21 = cat(blk(top2, 16)), cat(blk(bot2, 0))
                sums = [v.astype(BF16) for v in
                        _lhs_sums(*[v.astype(F32) for v in (a11, a12, a21, a22)])]
                m1 = _dot(sums[0], _ld(wos_s, 0))
                m2 = _dot(sums[1], _ld(wos_s, 1))
                m5 = _dot(sums[2], _ld(wos_s, 4))
                m6 = _dot(sums[3], _ld(wos_s, 5))
                m7 = _dot(sums[4], _ld(wos_s, 6))
                cs = (((m1 + m4) - m5) + m7, m3 + m5, m2 + m4, ((m1 - m2) + m3) + m6)
                for cb, rows, c0 in zip(cs, (top, top, bot, bot), (0, 512, 0, 512)):
                    oa_s[rows, c0:c0 + 512] = cb.astype(BF16)
                for v in range(NCT * 8 // nch):
                    u = i * (NCT * 8 // nch) + v
                    _b_s_pass3(zs_s, xre_s, xim_s, u // 8, u % 8, True)
                for cp in ocopies(i):
                    cp.start()
                return c
            lax.fori_loop(0, nch, ochunk, 0)

            copy(gdi_hbm, gdi_s, 8).wait()
            copy(gni_hbm, gni_s, 9).wait()

            def dinv(i, c):
                for a in range(BR // DSUB2):
                    r = pl.multiple_of(i * BR + a * DSUB2, DSUB2)
                    _b_d_inverse(xre_s, xim_s, gdi_s, gni_s, yb_s, r, DSUB2)
                for a in range(BR // DSUB2):
                    ycopy(i * (BR // DSUB2) + a).start()
                return c
            lax.fori_loop(0, S // BR, dinv, 0)
            for i in range(nch):
                for cp in ocopies(i):
                    cp.wait()
            for i in range(S // DSUB2):
                ycopy(i).wait()

        pl.run_scoped(a_out, pltpu.VMEM((S, DM), BF16), pltpu.VMEM((S, DM), BF16),
                      pltpu.VMEM((NCT, S, T), F32), pltpu.VMEM((NCT, S, T), F32),
                      pltpu.SemaphoreType.DMA((16 + S // DSUB2,)))

    pl.run_scoped(a_outer, pltpu.VMEM((H, S // 2, HD), U32), pltpu.VMEM((7, H * HD // 4, 512), U32))


@jax.jit
def pallas_concat_heads__compressed_kv_cla__spectral_gfnet__prompt_kernel(
    A_x, A_c_kv, A_w_q, A_w_uk, A_w_uv, A_w_o, B_x, B_w_r, B_w_i,
):
    hbm = pl.BlockSpec(memory_space=pl.ANY)
    out = pl.pallas_call(
        _kernel,
        in_specs=[hbm] * 15,
        out_specs=hbm,
        out_shape=jax.ShapeDtypeStruct((S, 2 * DM), BF16),
        scratch_shapes=[
            pltpu.VMEM((S, DM), BF16), pltpu.VMEM((S, DC), BF16),
            pltpu.VMEM((DM + 2 * DC + 2, 8, HD), BF16),
            pltpu.VMEM((H * HD + 16, DM), BF16),
            pltpu.VMEM((N1 + 1, NCT, T, T), BF16),
            pltpu.VMEM((4, 128, 256), U32), pltpu.VMEM((T // 2, T), U32),
            pltpu.SemaphoreType.DMA((10,)), pltpu.SemaphoreType.DMA((2 * NWO,)),
        ],
        compiler_params=pltpu.CompilerParams(vmem_limit_bytes=120 * 1024 * 1024),
    )(A_x.reshape(S, DM), A_c_kv.reshape(S, DC), A_w_q, A_w_uk, A_w_uv,
      A_w_o.reshape(H * HD, DM), B_x.reshape(S, DM), B_w_r.T, B_w_i.T, *_CONSTS)
    return out.reshape(1, S, 2 * DM)
```

```python
import functools
import math

import jax
import jax.numpy as jnp
import numpy as np
from jax import lax
from jax.experimental import pallas as pl
from jax.experimental.pallas import tpu as pltpu

S = 2048
DM = 1024
DC = 512
H = 32
HD = 128
T = 128
NG = 4
DF = DM // 2 + 1
NCT = 5
N1, N2 = 32, 64

F32, BF16, U32 = jnp.float32, jnp.bfloat16, jnp.uint32
LOG2E = math.log2(math.e)
Q_SCALE = float(HD ** -0.5 * LOG2E)
MASK_VAL = float(-1e9 * LOG2E)
CLASS_PAIRS = ((0, 4), (1, 7), (2, 6), (3, 5))


def _make_constants():
    b = np.arange(128)[:, None].astype(np.float64)
    m = np.arange(64)[None, :].astype(np.float64)

    def cs(r):
        th = 2.0 * np.pi * b * (r + 8.0 * m) / DM
        return np.cos(th), np.sin(th)

    gdf = np.zeros((4, 256, 256))
    c0, s0 = cs(0)
    c4, s4 = cs(4)
    gdf[0, :128, 0:64], gdf[0, :128, 128:192] = c0, -s0
    gdf[0, 128:, 64:128], gdf[0, 128:, 192:256] = c4, -s4
    for p in (1, 2, 3):
        r, r2 = CLASS_PAIRS[p]
        c, s = cs(r)
        c2, s2 = cs(r2)
        gdf[p, :128, 0:64], gdf[p, 128:, 0:64] = c, s
        gdf[p, :128, 64:128], gdf[p, 128:, 64:128] = c2, -s2
        gdf[p, :128, 128:192], gdf[p, 128:, 128:192] = -s, c
        gdf[p, :128, 192:256], gdf[p, 128:, 192:256] = -s2, -c2
    alt = (-1.0) ** np.arange(128)
    gnf = np.zeros((128, 128))
    gnf[:, 0] = alt

    sc = 1.0 / (S * DM)
    gdi = np.zeros((4, 256, 256))
    w0 = np.full((64, 1), 2.0)
    w0[0] = 1.0
    gdi[0, 0:64, 0:128] = (c0.T * w0) * sc
    gdi[0, 128:192, 0:128] = (-s0.T * w0) * sc
    gdi[0, 128, :] = 0.0
    gdi[0, 64:128, 128:256] = 2.0 * c4.T * sc
    gdi[0, 192:256, 128:256] = -2.0 * s4.T * sc
    for p in (1, 2, 3):
        r, r2 = CLASS_PAIRS[p]
        c, s = cs(r)
        c2, s2 = cs(r2)
        f = 2.0 * sc
        gdi[p, 0:64, 0:128], gdi[p, 128:192, 0:128] = f * c.T, -f * s.T
        gdi[p, 64:128, 0:128], gdi[p, 192:256, 0:128] = f * c2.T, -f * s2.T
        gdi[p, 0:64, 128:256], gdi[p, 128:192, 128:256] = f * s.T, f * c.T
        gdi[p, 64:128, 128:256], gdi[p, 192:256, 128:256] = -f * s2.T, -f * c2.T
    gni = np.zeros((128, 128))
    gni[0, :] = alt * sc

    n2 = np.arange(N2)
    perm = np.concatenate([np.concatenate([8 * j + np.arange(8), 64 + 8 * j + np.arange(8)])
                           for j in range(8)])
    gsf = np.zeros((N1, 128, 128))
    gsi = np.zeros((N1, 128, 128))
    for k1 in range(N1):
        k = k1 + N1 * n2
        g = np.exp(-2j * np.pi * np.outer(k, n2) / S)
        ghat = np.block([[g.real, -g.imag], [g.imag, g.real]])
        gsf[k1] = ghat[perm][:, perm]
        gsi[k1] = ghat.T[perm][:, perm]
    def words(a):
        u = np.asarray(a, dtype=np.float32).astype(jnp.bfloat16).view(np.uint16).astype(np.uint32)
        return np.ascontiguousarray(u[..., 0::2, :] | (u[..., 1::2, :] << 16))
    return tuple(words(a) for a in (gdf, gnf, gdi, gni, gsf, gsi))


_CONSTS = _make_constants()


def _dot(a, b):
    return jnp.dot(a, b, preferred_element_type=F32)


def _dot_nt(a, b):
    return lax.dot_general(a, b, (((1,), (1,)), ((), ())), preferred_element_type=F32)


def _ld(ref, *idx):
    return pltpu.bitcast(ref[idx], BF16)


def _pk(v):
    return pltpu.bitcast(v.astype(BF16), U32)


def _rows(r0, n):
    return pl.ds(r0 // 2, n // 2)


def _cmul_const(x, e, n, sign):
    re, im = x
    e %= n
    if e == 0:
        return re, im
    if 8 * e % n == 0:
        o = 8 * e // n
        if sign < 0:
            o = (8 - o) % 8
        h = math.sqrt(0.5)
        if o == 2:
            return -im, re
        if o == 4:
            return -re, -im
        if o == 6:
            return im, -re
        if o == 1:
            return (re - im) * h, (re + im) * h
        if o == 3:
            return (re + im) * (-h), (re - im) * h
        if o == 5:
            return (im - re) * h, (re + im) * (-h)
        if o == 7:
            return (re + im) * h, (im - re) * h
    th = sign * 2.0 * math.pi * e / n
    c, s = math.cos(th), math.sin(th)
    return re * c - im * s, re * s + im * c


def _cadd(a, b):
    return a[0] + b[0], a[1] + b[1]


def _csub(a, b):
    return a[0] - b[0], a[1] - b[1]


def _fft(xs, sign):
    n = len(xs)
    if n == 1:
        return xs
    if n == 2:
        return [_cadd(xs[0], xs[1]), _csub(xs[0], xs[1])]
    u = _fft(xs[0::2], sign)
    z1 = _fft(xs[1::4], sign)
    z3 = _fft(xs[3::4], sign)
    out = [None] * n
    q = n // 4
    for k in range(q):
        a = _cmul_const(z1[k], k, n, sign)
        b = _cmul_const(z3[k], 3 * k, n, sign)
        sm, df = _cadd(a, b), _csub(a, b)
        out[k] = _cadd(u[k], sm)
        out[k + 2 * q] = _csub(u[k], sm)
        if sign < 0:
            out[k + q] = (u[k + q][0] + df[1], u[k + q][1] - df[0])
            out[k + 3 * q] = (u[k + q][0] - df[1], u[k + q][1] + df[0])
        else:
            out[k + q] = (u[k + q][0] - df[1], u[k + q][1] + df[0])
            out[k + 3 * q] = (u[k + q][0] + df[1], u[k + q][1] - df[0])
    return out


def _b_words(a, b):
    return (pltpu.bitcast(a.astype(F32), U32) >> 16) | (
        pltpu.bitcast(b.astype(F32), U32) & jnp.uint32(0xFFFF0000))


def _b_prepare_w_words(wrT_s, wiT_s, wd_s, t):
    cols = pl.ds(pl.multiple_of(t * T, T), T)
    for a in range(0, 512, 64):
        wd_s[t, a:a + 64, :] = _b_words(wrT_s[a:a + 64, cols], wiT_s[a:a + 64, cols])


def _b_prepare_w_order(wrT_s, wiT_s, wd_s, wt_s, t):
    rows = pl.ds(pl.multiple_of(t * T, T), T)
    for p, (r, r2) in enumerate(CLASS_PAIRS):
        a = wd_s[t, pl.ds(r, 64, stride=8), :]
        b = wd_s[t, pl.ds(r2, 64, stride=8), :]
        wt_s[p, rows, :] = jnp.concatenate([a, b], axis=0).T
    ny = _b_words(wrT_s[512:513, rows], wiT_s[512:513, rows])
    row = lax.broadcasted_iota(jnp.int32, (T, T), 0)
    wt_s[4, rows, :] = jnp.where(row == 0, jnp.broadcast_to(ny, (T, T)), jnp.uint32(0)).T


def _b_d_forward_vpu(xb_s, y_s, slot, r0, rows):
    for a in range(0, rows, VSL):
        _b_d_forward_vpu_slab(xb_s, y_s, slot, r0, a)


def _b_d_forward_vpu_slab(xb_s, y_s, slot, r0, a):
    sl = pl.ds(r0 + a, VSL)
    x = [xb_s[sl, a * T:(a + 1) * T].astype(F32) for a in range(8)]
    s04, t = x[0] + x[4], x[0] - x[4]
    s26, u = x[2] + x[6], x[2] - x[6]
    s15, v = x[1] + x[5], x[1] - x[5]
    s37, w = x[3] + x[7], x[3] - x[7]
    e, f = s04 + s26, s04 - s26
    g, hh = s15 + s37, s15 - s37
    k = math.sqrt(0.5)
    al, be = (v - w) * k, (v + w) * k
    ys = ((e + g, e - g),
          (t + al, -(u + be)),
          (f, -hh),
          (t - al, u - be))
    for p in range(4):
        y_s[slot, a // 2:(a + VSL) // 2, 2 * p * T:(2 * p + 2) * T] = _pk(jnp.concatenate(
            [ys[p][0], ys[p][1]], axis=1))


def _b_d_forward_mxu(y_s, slot, gdf_s, gnf_s, xre_s, xim_s, r0, a, rows):
    sl = pl.ds(r0 + a, rows)
    for p in range(4):
        o = _dot(_ld(y_s, slot, slice(a // 2, (a + rows) // 2), slice(2 * p * T, (2 * p + 2) * T)), _ld(gdf_s, p))
        xre_s[p, sl, :] = o[:, :T]
        xim_s[p, sl, :] = o[:, T:]
    xre_s[4, sl, :] = _dot(_ld(y_s, slot, slice(a // 2, (a + rows) // 2), slice(0, T)),
                           pltpu.bitcast(gnf_s[...], BF16))
    xim_s[4, sl, :] = jnp.zeros((rows, T), F32)


def _fft32(load, emit, sign):
    half = N1 // 2
    for par in range(2):
        xs = []
        for n in range(half):
            a, b = load(n), load(n + half)
            xs.append(_cadd(a, b) if par == 0 else _cmul_const(_csub(a, b), n, N1, sign))
        out = _fft(xs, sign)
        for q in range(half):
            emit(2 * q + par, out[q])


def _b_s_pass1(xre_s, xim_s, ys_s, c, j):
    off = pl.multiple_of(j * 8, 8)

    def load(n1):
        rows = pl.ds(N2 * n1 + off, 8)
        return xre_s[c, rows, :], xim_s[c, rows, :]

    def emit(k1, v):
        ys_s[k1, c, pl.ds(pl.multiple_of(j * 16, 16), 16), :] = jnp.concatenate(v, axis=0).astype(BF16)
    _fft32(load, emit, -1)


def _b_s_pass2_fwd(ys_s, gsf_s, k1):
    rhs = jnp.concatenate([ys_s[k1, c] for c in range(NCT)], axis=1)
    return _dot(_ld(gsf_s, k1), rhs)


def _b_s_pass2_inv(vv, zs_s, wt_s, gsi_s, k1):
    outs = []
    for c in range(NCT):
        wd = wt_s[c, pl.ds(k1, N2, stride=N1), :]
        wr = pltpu.bitcast(wd << 16, F32)
        wi = pltpu.bitcast(wd & jnp.uint32(0xFFFF0000), F32)
        pcs = []
        for j in range(8):
            vr = vv[16 * j:16 * j + 8, c * T:(c + 1) * T]
            vi = vv[16 * j + 8:16 * j + 16, c * T:(c + 1) * T]
            a, b = wr[8 * j:8 * j + 8], wi[8 * j:8 * j + 8]
            pcs.append(vr * a - vi * b)
            pcs.append(vr * b + vi * a)
        outs.append(jnp.concatenate(pcs, axis=0).astype(BF16))
    ginv = _ld(gsi_s, k1)
    for c in range(NCT):
        zs_s[k1, c] = _dot(ginv, outs[c]).astype(BF16)


def _b_s_pass2(ys_s, zs_s, wt_s, gsf_s, gsi_s, k1s):
    pend = []
    for a in range(len(k1s) + P2D):
        if a < len(k1s):
            pend.append(_b_s_pass2_fwd(ys_s, gsf_s, k1s[a]))
        if a >= P2D:
            _b_s_pass2_inv(pend.pop(0), zs_s, wt_s, gsi_s, k1s[a - P2D])


def _b_s_pass3(zs_s, xre_s, xim_s, c, j, chain):
    off = pl.multiple_of(j * 8, 8)

    def load(k1):
        z = zs_s[k1, c, pl.ds(pl.multiple_of(j * 16, 16), 16), :].astype(F32)
        return z[0:8], z[8:16]

    def emit(n1, v):
        rows = pl.ds(N2 * n1 + off, 8)
        xre_s[c, rows, :] = v[0]
        xim_s[c, rows, :] = v[1]
        if chain and n1 >= N1 - 2:
            zs_s[N1, 0, 0:16, :] = jnp.concatenate(v, axis=0).astype(BF16)
    _fft32(load, emit, +1)


def _b_d_inverse(xre_s, xim_s, gdi_s, gni_s, yb_s, r0, rows):
    sl = pl.ds(r0, rows)
    us = []
    for p in range(4):
        lhs = jnp.concatenate([xre_s[p, sl, :], xim_s[p, sl, :]], axis=1).astype(BF16)
        o = _dot(lhs, _ld(gdi_s, p))
        us.append((o[:, :T], o[:, T:]))
    u0 = us[0][0] + _dot(xre_s[4, sl, :].astype(BF16), pltpu.bitcast(gni_s[...], BF16))
    u4 = us[0][1]
    (u1r, u1i), (u2r, u2i), (u3r, u3i) = us[1], us[2], us[3]
    e0, e1 = u0 + u4, u0 - u4
    ev = (e0 + u2r, e1 - u2i, e0 - u2r, e1 + u2i)
    pq, qq = u1r - u3r, u1i + u3i
    k = math.sqrt(0.5)
    od = (u1r + u3r, (pq - qq) * k, u3i - u1i, (pq + qq) * (-k))
    for a in range(4):
        yb_s[sl, a * T:(a + 1) * T] = (ev[a] + od[a]).astype(BF16)
        yb_s[sl, (a + 4) * T:(a + 5) * T] = (ev[a] - od[a]).astype(BF16)


VSL = 16
BQ = 128
ADEPTH = 2
ACK = 128
AORD = 3
AUN = 2


def _attn_order(h0):
    n = S // BQ
    if AORD == 0:
        return [(h0 + u, i) for u in range(AUN) for i in range(n - 1, -1, -1)]
    if AORD == 1:
        return [p for i in range(n) for p in ((h0, n - 1 - i), (h0 + 1, i))]
    if AORD >= 2:
        o = []
        lo, hi = 0, n - 1
        while lo <= hi:
            o.append(hi)
            hi -= 1
            if lo <= hi:
                o.append(lo)
                lo += 1
        if AORD == 2:
            return [(h0 + u, i) for u in range(AUN) for i in o]
        if AORD == 3:
            return [(h0 + u, i) for i in o for u in range(AUN)]
        if AORD == 4:
            return [(h0, i) for i in o] + [(h0 + 1, i) for i in o[::-1]]
        if AORD == 5:
            return [p for a, b in zip(o, o[::-1]) for p in ((h0, a), (h0 + 1, b))]


def _attn_heads(q_s, k_s, v_s, o_s, h0, ho):
    nt = BQ // T
    row = lax.broadcasted_iota(jnp.int32, (T, T), 0)
    col = lax.broadcasted_iota(jnp.int32, (T, T), 1)
    causal = col <= row

    def scores(h, i):
        r0 = i * BQ
        nfull = r0 // T + 1
        tiles = {}
        s = _dot_nt(_ld(q_s, h, _rows(r0, BQ)), _ld(k_s, h, _rows(0, nfull * T)))
        for t in range(nt):
            for j in range(nfull):
                tiles[t, j] = s[t * T:(t + 1) * T, j * T:(j + 1) * T]
        for t in range(1, nt):
            j = nfull - 1 + t
            st = _dot_nt(_ld(q_s, h, _rows(r0 + t * T, BQ - t * T)), _ld(k_s, h, _rows(j * T, T)))
            for u in range(t, nt):
                tiles[u, j] = st[(u - t) * T:(u - t + 1) * T]
        for t in range(nt):
            jd = nfull - 1 + t
            tiles[t, jd] = jnp.where(causal, tiles[t, jd], MASK_VAL)
        return tiles

    def softmax_pv(h, i, tiles):
        r0 = i * BQ
        nfull = r0 // T + 1
        for t in range(nt):
            nk = nfull + t
            mx = tiles[t, 0]
            for j in range(1, nk):
                mx = jnp.maximum(mx, tiles[t, j])
            m = jnp.max(mx, axis=1, keepdims=True)
            lacc = o = None
            cj = ACK // T
            for j0 in range(0, nk, cj):
                ps = []
                for j in range(j0, min(nk, j0 + cj)):
                    p = jnp.exp2(tiles[t, j] - m)
                    lacc = p if lacc is None else lacc + p
                    ps.append(p)
                pc = jnp.concatenate(ps, axis=1) if len(ps) > 1 else ps[0]
                oo = _dot(pc.astype(BF16), _ld(v_s, h, _rows(j0 * T, len(ps) * T)))
                o = oo if o is None else o + oo
            l = jnp.sum(lacc, axis=1, keepdims=True)
            o_s[h - h0 + ho, _rows(r0 + t * T, T)] = _pk(o * pl.reciprocal(l, approx=True))

    order = _attn_order(h0)
    pend = []
    for a in range(len(order) + ADEPTH):
        if a < len(order):
            pend.append(scores(*order[a]))
        if a >= ADEPTH:
            softmax_pv(*order[a - ADEPTH], pend.pop(0))


HS = S // 2


def _lhs_sums(a11, a12, a21, a22):
    return (a11 + a22, a21 + a22, a11 + a12, a21 - a11, a12 - a22)


def _rhs_ops(b11, b12, b21, b22):
    return (b11 + b22, b11, b12 - b22, b21 - b11, b22, b11 + b12, b21 + b22)


def _strassen(lhs, rhs):
    m3, m4 = _dot(lhs[2], rhs[2]), _dot(lhs[3], rhs[3])
    m1, m2, m5, m6, m7 = [_dot(lhs[j], rhs[j]) for j in (0, 1, 4, 5, 6)]
    return (((m1 + m4) - m5) + m7, m3 + m5, m2 + m4, ((m1 - m2) + m3) + m6)


PR = 256
OR = 128
BR = 512
DSUB = 64
P2D = 1
P2U = 8
WSL = 16
WSL2 = 32
OCH = 1
AREP = 1
DMA_A = 4
DMA_B = 32
DSUB2 = 128
WPIN = 0
PORD = 3
WORD = 3
NWO = 16


def _kernel(ax_hbm, ac_hbm, wq_hbm, wuk_hbm, wuv_hbm, wo_hbm, bx_hbm, wrT_hbm, wiT_hbm,
            gdf_hbm, gnf_hbm, gdi_hbm, gni_hbm, gsf_hbm, gsi_hbm,
            out_hbm,
            ax_s, ac_s, w_st, wo_s, zs_s, gdi_s, gni_s, sems, wosem):
    def copy(src, dst, i):
        return pltpu.make_async_copy(src, dst, sems.at[i])

    def wcopies(g):
        hs = pl.ds(pl.multiple_of(g * 8, 8), 8)
        return (copy(wq_hbm.at[:, hs, :], w_st.at[pl.ds(0, DM)], 2),
                copy(wuk_hbm.at[:, hs, :], w_st.at[pl.ds(DM, DC)], 3),
                copy(wuv_hbm.at[:, hs, :], w_st.at[pl.ds(DM + DC, DC)], 4))

    def wocopies(u):
        r = pl.multiple_of(u * T, T)
        r2 = pl.multiple_of(H * HD // 2 + u * T, T)
        return (pltpu.make_async_copy(wo_hbm.at[pl.ds(r, T), :], wo_s.at[pl.ds(r, T), :], wosem.at[2 * u]),
                pltpu.make_async_copy(wo_hbm.at[pl.ds(r2, T), :], wo_s.at[pl.ds(r2, T), :], wosem.at[2 * u + 1]))

    def b_phase(bx_s, y_s, wrT_s, wiT_s, wd_s, wt_s, xre_s, xim_s, ys_s,
                gdf_s, gnf_s, gsf_s, gsi_s, bsem):
        def bcopy(src, dst, i):
            return pltpu.make_async_copy(src, dst, bsem.at[i])
        nch = S // BR
        xc = [bcopy(bx_hbm.at[pl.ds(i * BR, BR), :], bx_s.at[pl.ds(i * BR, BR), :], i)
              for i in range(nch)]
        cc = [bcopy(gdf_hbm, gdf_s, nch), bcopy(gnf_hbm, gnf_s, nch + 1),
              bcopy(wrT_hbm, wrT_s, nch + 2), bcopy(wiT_hbm, wiT_s, nch + 3),
              bcopy(gsf_hbm, gsf_s, nch + 4), bcopy(gsi_hbm, gsi_s, nch + 5)]
        xc[0].start()
        cc[0].start()
        cc[1].start()
        xc[1].start()

        cc[0].wait()
        cc[1].wait()
        xc[0].wait()
        xc[2].start()
        _b_d_forward_vpu(bx_s, y_s, 0, 0, BR)

        for i in range(nch):
            if i + 1 < nch:
                xc[i + 1].wait()
            if i == 0:
                xc[3].start()
            if i == 2:
                cc[2].start()
                cc[3].start()
            for a in range(0, BR, DSUB):
                _b_d_forward_mxu(y_s, i % 2, gdf_s, gnf_s, xre_s, xim_s, i * BR, a, DSUB)
                if i + 1 < nch:
                    for b in range(a, a + DSUB, VSL):
                        _b_d_forward_vpu_slab(bx_s, y_s, (i + 1) % 2, (i + 1) * BR, b)

        cc[2].wait()
        cc[3].wait()
        cc[4].start()
        cc[5].start()
        copy(ac_hbm, ac_s, 1).start()

        def p1(i, c):
            @pl.when(i == DMA_A)
            def _():
                copy(ax_hbm, ax_s, 0).start()
            for v in range(2):
                _b_prepare_w_order(wrT_s, wiT_s, wd_s, wt_s, 2 * i + v)
            for v in range(NCT):
                u = i * NCT + v
                _b_s_pass1(xre_s, xim_s, ys_s, u // 8, u % 8)
            for v in range(2):
                _b_prepare_w_words(wrT_s, wiT_s, wd_s, jnp.minimum(2 * i + 2 + v, S // T - 1))
            return c
        for v in range(2):
            _b_prepare_w_words(wrT_s, wiT_s, wd_s, v)
        lax.fori_loop(0, 8, p1, 0)
        cc[4].wait()
        cc[5].wait()
        copy(ac_hbm, ac_s, 1).wait()
        for cp in wcopies(0):
            cp.start()

        npi = N1 // P2U

        def p2(kk, c):
            @pl.when(kk == npi - 1)
            def _():
                for v in range(NWO):
                    for cp in wocopies(v):
                        cp.start()
                copy(gdi_hbm, gdi_s, 8).start()
                copy(gni_hbm, gni_s, 9).start()
            _b_s_pass2(ys_s, zs_s, wt_s, gsf_s, gsi_s, [kk * P2U + u for u in range(P2U)])
            return c
        lax.fori_loop(0, N1 // P2U, p2, 0)

    def b_scope():
      pl.run_scoped(
        b_phase,
        pltpu.VMEM((S, DM), BF16), pltpu.VMEM((2, BR // 2, DM), U32),
        pltpu.VMEM((DF, S), BF16), pltpu.VMEM((DF, S), BF16),
        pltpu.VMEM((S // T, 512, T), U32), pltpu.VMEM((NCT, S, T), U32),
        pltpu.VMEM((NCT, S, T), F32), pltpu.VMEM((NCT, S, T), F32),
        pltpu.VMEM((N1, NCT, T, T), BF16),
        pltpu.VMEM((4, 128, 256), U32), pltpu.VMEM((T // 2, T), U32),
        pltpu.VMEM((N1, T // 2, T), U32), pltpu.VMEM((N1, T // 2, T), U32),
        pltpu.SemaphoreType.DMA((S // BR + 6,)),
    )

    def a_outer(ctx_s, wos_s):
        def a_main(wu_s, q_s, k_s, v_s):
            def stage_w(i, chain):
                rows = (DM + 2 * DC) // 8
                step = WSL2 if chain else 128
                for a in range(0, rows, step):
                    r = pl.multiple_of(i * rows + a, step)
                    v = w_st[pl.ds(r, step)]
                    wu_s[pl.ds(pl.multiple_of(4 * r, 4 * step), 4 * step), :] = pltpu.bitcast(
                        v.reshape(step * 8, HD), U32)
                    if chain:
                        w_st[DM + 2 * DC:DM + 2 * DC + 2] = v[0:2]

            def w_rhs(slot, base, kk):
                def blk(m0, hp0):
                    cols = []
                    for hp in (hp0, hp0 + 1):
                        x = wu_s[pl.ds(4 * m0 + hp, kk, stride=4), :]
                        cols.append(pltpu.bitcast(x << 16, F32))
                        cols.append(pltpu.bitcast(x & jnp.uint32(0xFFFF0000), F32))
                    return jnp.concatenate(cols, axis=1)
                b11, b12 = blk(base, 0), blk(base, 2)
                b21, b22 = blk(base + kk, 0), blk(base + kk, 2)
                return [v.astype(BF16) for v in _rhs_ops(b11, b12, b21, b22)]

            def prep_wo(u, chain):
                step = WSL if chain else T
                for a in range(0, T, step):
                    r = pl.multiple_of(u * T + a, step)
                    top = wo_s[pl.ds(r, step), :].astype(F32)
                    bot = wo_s[pl.ds(H * HD // 2 + r, step), :].astype(F32)
                    ops = _rhs_ops(top[:, :512], top[:, 512:], bot[:, :512], bot[:, 512:])
                    r2 = pl.multiple_of(u * (T // 2) + a // 2, step // 2)
                    for j in range(7):
                        v = ops[j].astype(BF16)
                        wos_s[j, pl.ds(r2, step // 2), :] = pltpu.bitcast(v, U32)
                    if chain:
                        wo_s[H * HD:H * HD + 16, 0:HD] = v[0:16, 0:HD]

            copy(ax_hbm, ax_s, 0).wait()
            for cp in wcopies(0):
                cp.wait()

            def prew(i, c):
                stage_w(i, False)
                return c
            lax.fori_loop(0, 8, prew, 0)

            def lhs7(src, r):
                kk = src.shape[1] // 2
                top, bot = pl.ds(r, PR), pl.ds(HS + r, PR)
                a11, a12, a21, a22 = src[top, :kk], src[top, kk:], src[bot, :kk], src[bot, kk:]
                sm = [v.astype(BF16) for v in _lhs_sums(*[v.astype(F32) for v in (a11, a12, a21, a22)])]
                return (sm[0], sm[1], a11, a22, sm[2], sm[3], sm[4])

            def group(g, c):
                slot = 0
                gn = jnp.minimum(g + 1, NG - 1)
                for cp in wcopies(gn):
                    cp.start()

                def chunk(i, cc):
                    r = pl.multiple_of(i * PR, PR)
                    top, bot = pl.ds(r, PR), pl.ds(HS + r, PR)
                    for cp in wocopies(g * 4 + i):
                        cp.wait()

                    def put(dst, cs, scale=None):
                        top2 = pl.ds(pl.multiple_of(i * (PR // 2), PR // 2), PR // 2)
                        bot2 = pl.ds(pl.multiple_of(HS // 2 + i * (PR // 2), PR // 2), PR // 2)
                        for cb, rows, h0 in zip(cs, (top2, top2, bot2, bot2), (0, 4, 0, 4)):
                            if scale is not None:
                                cb = cb * scale
                            cb = _pk(cb)
                            for hh in range(4):
                                dst[h0 + hh, rows, :] = cb[:, hh * HD:(hh + 1) * HD]
                    cl = lhs7(ac_s, r)
                    kcs = _strassen(cl, w_rhs(slot, DM, DC // 2))
                    put(k_s, kcs)
                    if WPIN == 1:
                        wo_s[H * HD:H * HD + 16, 0:HD] = kcs[1][0:16, 0:HD].astype(BF16)
                        prep_wo(g * 4 + i, True)
                    put(v_s, _strassen(cl, w_rhs(slot, DM + DC, DC // 2)))
                    put(q_s, _strassen(lhs7(ax_s, r), w_rhs(slot, 0, DM // 2)), Q_SCALE)
                    if WPIN == 0: prep_wo(g * 4 + i, True)
                    return cc
                lax.fori_loop(0, HS // PR, chunk, 0)

                for cp in wcopies(gn):
                    cp.wait()

                def head(hh, cc):
                    h = hh * AUN
                    _attn_heads(q_s, k_s, v_s, ctx_s, h, g * 8 + h)
                    for u in range(AUN):
                        stage_w(h + u, True)
                    return cc
                lax.fori_loop(0, 8 // AUN, head, 0)
                return c
            lax.fori_loop(0, NG, group, 0)

        b_scope()
        pl.run_scoped(a_main, pltpu.VMEM((4 * (DM + 2 * DC), HD), U32),
                      *[pltpu.VMEM((8, S // 2, HD), U32)] * 3)

        def a_out(oa_s, yb_s, xre_s, xim_s, osem):
            nch = HS // OR

            def ocopies(i):
                r = pl.multiple_of(i * OR, OR)
                r2 = pl.multiple_of(HS + i * OR, OR)
                return (pltpu.make_async_copy(oa_s.at[pl.ds(r, OR), :],
                                              out_hbm.at[pl.ds(r, OR), pl.ds(0, DM)], osem.at[2 * i]),
                        pltpu.make_async_copy(oa_s.at[pl.ds(r2, OR), :],
                                              out_hbm.at[pl.ds(r2, OR), pl.ds(0, DM)], osem.at[2 * i + 1]))

            def ycopy(i):
                r = pl.multiple_of(i * DSUB2, DSUB2)
                return pltpu.make_async_copy(yb_s.at[pl.ds(r, DSUB2), :],
                                             out_hbm.at[pl.ds(r, DSUB2), pl.ds(DM, DM)], osem.at[16 + i])

            def blk(rows, h0):
                return [_ld(ctx_s, h0 + h, rows) for h in range(H // 2)]

            def ochunk(i, c):
                r = pl.multiple_of(i * OR, OR)
                top, bot = pl.ds(r, OR), pl.ds(HS + r, OR)
                cat = lambda xs: jnp.concatenate(xs, axis=1)
                hk = H * HD // 2
                top2 = pl.ds(pl.multiple_of(i * (OR // 2), OR // 2), OR // 2)
                bot2 = pl.ds(pl.multiple_of(HS // 2 + i * (OR // 2), OR // 2), OR // 2)
                a11, a22 = cat(blk(top2, 0)), cat(blk(bot2, 16))
                m3 = _dot(a11, _ld(wos_s, 2))
                m4 = _dot(a22, _ld(wos_s, 3))
                a12, a21 = cat(blk(top2, 16)), cat(blk(bot2, 0))
                sums = [v.astype(BF16) for v in
                        _lhs_sums(*[v.astype(F32) for v in (a11, a12, a21, a22)])]
                m1 = _dot(sums[0], _ld(wos_s, 0))
                m2 = _dot(sums[1], _ld(wos_s, 1))
                m5 = _dot(sums[2], _ld(wos_s, 4))
                m6 = _dot(sums[3], _ld(wos_s, 5))
                m7 = _dot(sums[4], _ld(wos_s, 6))
                cs = (((m1 + m4) - m5) + m7, m3 + m5, m2 + m4, ((m1 - m2) + m3) + m6)
                for cb, rows, c0 in zip(cs, (top, top, bot, bot), (0, 512, 0, 512)):
                    oa_s[rows, c0:c0 + 512] = cb.astype(BF16)
                for v in range(NCT * 8 // nch):
                    u = i * (NCT * 8 // nch) + v
                    _b_s_pass3(zs_s, xre_s, xim_s, u // 8, u % 8, True)
                for cp in ocopies(i):
                    cp.start()
                return c
            lax.fori_loop(0, nch, ochunk, 0)

            copy(gdi_hbm, gdi_s, 8).wait()
            copy(gni_hbm, gni_s, 9).wait()

            def dinv(i, c):
                for a in range(BR // DSUB2):
                    r = pl.multiple_of(i * BR + a * DSUB2, DSUB2)
                    _b_d_inverse(xre_s, xim_s, gdi_s, gni_s, yb_s, r, DSUB2)
                for a in range(BR // DSUB2):
                    ycopy(i * (BR // DSUB2) + a).start()
                return c
            lax.fori_loop(0, S // BR, dinv, 0)
            for i in range(nch):
                for cp in ocopies(i):
                    cp.wait()
            for i in range(S // DSUB2):
                ycopy(i).wait()

        pl.run_scoped(a_out, pltpu.VMEM((S, DM), BF16), pltpu.VMEM((S, DM), BF16),
                      pltpu.VMEM((NCT, S, T), F32), pltpu.VMEM((NCT, S, T), F32),
                      pltpu.SemaphoreType.DMA((16 + S // DSUB2,)))

    pl.run_scoped(a_outer, pltpu.VMEM((H, S // 2, HD), U32), pltpu.VMEM((7, H * HD // 4, 512), U32))


@jax.jit
def pallas_concat_heads__compressed_kv_cla__spectral_gfnet__prompt_kernel(
    A_x, A_c_kv, A_w_q, A_w_uk, A_w_uv, A_w_o, B_x, B_w_r, B_w_i,
):
    hbm = pl.BlockSpec(memory_space=pl.ANY)
    out = pl.pallas_call(
        _kernel,
        in_specs=[hbm] * 15,
        out_specs=hbm,
        out_shape=jax.ShapeDtypeStruct((S, 2 * DM), BF16),
        scratch_shapes=[
            pltpu.VMEM((S, DM), BF16), pltpu.VMEM((S, DC), BF16),
            pltpu.VMEM((DM + 2 * DC + 2, 8, HD), BF16),
            pltpu.VMEM((H * HD + 16, DM), BF16),
            pltpu.VMEM((N1 + 1, NCT, T, T), BF16),
            pltpu.VMEM((4, 128, 256), U32), pltpu.VMEM((T // 2, T), U32),
            pltpu.SemaphoreType.DMA((10,)), pltpu.SemaphoreType.DMA((2 * NWO,)),
        ],
        compiler_params=pltpu.CompilerParams(vmem_limit_bytes=120 * 1024 * 1024),
    )(A_x.reshape(S, DM), A_c_kv.reshape(S, DC), A_w_q, A_w_uk, A_w_uv,
      A_w_o.reshape(H * HD, DM), B_x.reshape(S, DM), B_w_r.T, B_w_i.T, *_CONSTS)
    return out.reshape(1, S, 2 * DM)
```

```python
import functools
import math

import jax
import jax.numpy as jnp
import numpy as np
from jax import lax
from jax.experimental import pallas as pl
from jax.experimental.pallas import tpu as pltpu

S = 2048
DM = 1024
DC = 512
H = 32
HD = 128
T = 128
NG = 4
DF = DM // 2 + 1
NCT = 5
N1, N2 = 32, 64

F32, BF16, U32 = jnp.float32, jnp.bfloat16, jnp.uint32
LOG2E = math.log2(math.e)
Q_SCALE = float(HD ** -0.5 * LOG2E)
MASK_VAL = float(-1e9 * LOG2E)
CLASS_PAIRS = ((0, 4), (1, 7), (2, 6), (3, 5))


def _make_constants():
    b = np.arange(128)[:, None].astype(np.float64)
    m = np.arange(64)[None, :].astype(np.float64)

    def cs(r):
        th = 2.0 * np.pi * b * (r + 8.0 * m) / DM
        return np.cos(th), np.sin(th)

    gdf = np.zeros((4, 256, 256))
    c0, s0 = cs(0)
    c4, s4 = cs(4)
    gdf[0, :128, 0:64], gdf[0, :128, 128:192] = c0, -s0
    gdf[0, 128:, 64:128], gdf[0, 128:, 192:256] = c4, -s4
    for p in (1, 2, 3):
        r, r2 = CLASS_PAIRS[p]
        c, s = cs(r)
        c2, s2 = cs(r2)
        gdf[p, :128, 0:64], gdf[p, 128:, 0:64] = c, s
        gdf[p, :128, 64:128], gdf[p, 128:, 64:128] = c2, -s2
        gdf[p, :128, 128:192], gdf[p, 128:, 128:192] = -s, c
        gdf[p, :128, 192:256], gdf[p, 128:, 192:256] = -s2, -c2
    alt = (-1.0) ** np.arange(128)
    gnf = np.zeros((128, 128))
    gnf[:, 0] = alt

    sc = 1.0 / (S * DM)
    gdi = np.zeros((4, 256, 256))
    w0 = np.full((64, 1), 2.0)
    w0[0] = 1.0
    gdi[0, 0:64, 0:128] = (c0.T * w0) * sc
    gdi[0, 128:192, 0:128] = (-s0.T * w0) * sc
    gdi[0, 128, :] = 0.0
    gdi[0, 64:128, 128:256] = 2.0 * c4.T * sc
    gdi[0, 192:256, 128:256] = -2.0 * s4.T * sc
    for p in (1, 2, 3):
        r, r2 = CLASS_PAIRS[p]
        c, s = cs(r)
        c2, s2 = cs(r2)
        f = 2.0 * sc
        gdi[p, 0:64, 0:128], gdi[p, 128:192, 0:128] = f * c.T, -f * s.T
        gdi[p, 64:128, 0:128], gdi[p, 192:256, 0:128] = f * c2.T, -f * s2.T
        gdi[p, 0:64, 128:256], gdi[p, 128:192, 128:256] = f * s.T, f * c.T
        gdi[p, 64:128, 128:256], gdi[p, 192:256, 128:256] = -f * s2.T, -f * c2.T
    gni = np.zeros((128, 128))
    gni[0, :] = alt * sc

    n2 = np.arange(N2)
    perm = np.concatenate([np.concatenate([8 * j + np.arange(8), 64 + 8 * j + np.arange(8)])
                           for j in range(8)])
    gsf = np.zeros((N1, 128, 128))
    gsi = np.zeros((N1, 128, 128))
    for k1 in range(N1):
        k = k1 + N1 * n2
        g = np.exp(-2j * np.pi * np.outer(k, n2) / S)
        ghat = np.block([[g.real, -g.imag], [g.imag, g.real]])
        gsf[k1] = ghat[perm][:, perm]
        gsi[k1] = ghat.T[perm][:, perm]
    def words(a):
        u = np.asarray(a, dtype=np.float32).astype(jnp.bfloat16).view(np.uint16).astype(np.uint32)
        return np.ascontiguousarray(u[..., 0::2, :] | (u[..., 1::2, :] << 16))
    return tuple(words(a) for a in (gdf, gnf, gdi, gni, gsf, gsi))


_CONSTS = _make_constants()


def _dot(a, b):
    return jnp.dot(a, b, preferred_element_type=F32)


def _dot_nt(a, b):
    return lax.dot_general(a, b, (((1,), (1,)), ((), ())), preferred_element_type=F32)


def _ld(ref, *idx):
    return pltpu.bitcast(ref[idx], BF16)


def _pk(v):
    return pltpu.bitcast(v.astype(BF16), U32)


def _rows(r0, n):
    return pl.ds(r0 // 2, n // 2)


def _cmul_const(x, e, n, sign):
    re, im = x
    e %= n
    if e == 0:
        return re, im
    if 8 * e % n == 0:
        o = 8 * e // n
        if sign < 0:
            o = (8 - o) % 8
        h = math.sqrt(0.5)
        if o == 2:
            return -im, re
        if o == 4:
            return -re, -im
        if o == 6:
            return im, -re
        if o == 1:
            return (re - im) * h, (re + im) * h
        if o == 3:
            return (re + im) * (-h), (re - im) * h
        if o == 5:
            return (im - re) * h, (re + im) * (-h)
        if o == 7:
            return (re + im) * h, (im - re) * h
    th = sign * 2.0 * math.pi * e / n
    c, s = math.cos(th), math.sin(th)
    return re * c - im * s, re * s + im * c


def _cadd(a, b):
    return a[0] + b[0], a[1] + b[1]


def _csub(a, b):
    return a[0] - b[0], a[1] - b[1]


def _fft(xs, sign):
    n = len(xs)
    if n == 1:
        return xs
    if n == 2:
        return [_cadd(xs[0], xs[1]), _csub(xs[0], xs[1])]
    u = _fft(xs[0::2], sign)
    z1 = _fft(xs[1::4], sign)
    z3 = _fft(xs[3::4], sign)
    out = [None] * n
    q = n // 4
    for k in range(q):
        a = _cmul_const(z1[k], k, n, sign)
        b = _cmul_const(z3[k], 3 * k, n, sign)
        sm, df = _cadd(a, b), _csub(a, b)
        out[k] = _cadd(u[k], sm)
        out[k + 2 * q] = _csub(u[k], sm)
        if sign < 0:
            out[k + q] = (u[k + q][0] + df[1], u[k + q][1] - df[0])
            out[k + 3 * q] = (u[k + q][0] - df[1], u[k + q][1] + df[0])
        else:
            out[k + q] = (u[k + q][0] - df[1], u[k + q][1] + df[0])
            out[k + 3 * q] = (u[k + q][0] + df[1], u[k + q][1] - df[0])
    return out


def _b_words(a, b):
    return (pltpu.bitcast(a.astype(F32), U32) >> 16) | (
        pltpu.bitcast(b.astype(F32), U32) & jnp.uint32(0xFFFF0000))


def _b_prepare_w_words(wrT_s, wiT_s, wd_s, t):
    cols = pl.ds(pl.multiple_of(t * T, T), T)
    for a in range(0, 512, 64):
        wd_s[t, a:a + 64, :] = _b_words(wrT_s[a:a + 64, cols], wiT_s[a:a + 64, cols])


def _b_prepare_w_order(wrT_s, wiT_s, wd_s, wt_s, t):
    rows = pl.ds(pl.multiple_of(t * T, T), T)
    for p, (r, r2) in enumerate(CLASS_PAIRS):
        a = wd_s[t, pl.ds(r, 64, stride=8), :]
        b = wd_s[t, pl.ds(r2, 64, stride=8), :]
        wt_s[p, rows, :] = jnp.concatenate([a, b], axis=0).T
    ny = _b_words(wrT_s[512:513, rows], wiT_s[512:513, rows])
    row = lax.broadcasted_iota(jnp.int32, (T, T), 0)
    wt_s[4, rows, :] = jnp.where(row == 0, jnp.broadcast_to(ny, (T, T)), jnp.uint32(0)).T


def _b_d_forward_vpu(xb_s, y_s, slot, r0, rows):
    for a in range(0, rows, VSL):
        _b_d_forward_vpu_slab(xb_s, y_s, slot, r0, a)


def _b_d_forward_vpu_slab(xb_s, y_s, slot, r0, a):
    sl = pl.ds(r0 + a, VSL)
    x = [xb_s[sl, a * T:(a + 1) * T].astype(F32) for a in range(8)]
    s04, t = x[0] + x[4], x[0] - x[4]
    s26, u = x[2] + x[6], x[2] - x[6]
    s15, v = x[1] + x[5], x[1] - x[5]
    s37, w = x[3] + x[7], x[3] - x[7]
    e, f = s04 + s26, s04 - s26
    g, hh = s15 + s37, s15 - s37
    k = math.sqrt(0.5)
    al, be = (v - w) * k, (v + w) * k
    ys = ((e + g, e - g),
          (t + al, -(u + be)),
          (f, -hh),
          (t - al, u - be))
    for p in range(4):
        y_s[slot, a // 2:(a + VSL) // 2, 2 * p * T:(2 * p + 2) * T] = _pk(jnp.concatenate(
            [ys[p][0], ys[p][1]], axis=1))


def _b_d_forward_mxu(y_s, slot, gdf_s, gnf_s, xre_s, xim_s, r0, a, rows):
    sl = pl.ds(r0 + a, rows)
    for p in range(4):
        o = _dot(_ld(y_s, slot, slice(a // 2, (a + rows) // 2), slice(2 * p * T, (2 * p + 2) * T)), _ld(gdf_s, p))
        xre_s[p, sl, :] = o[:, :T]
        xim_s[p, sl, :] = o[:, T:]
    xre_s[4, sl, :] = _dot(_ld(y_s, slot, slice(a // 2, (a + rows) // 2), slice(0, T)),
                           pltpu.bitcast(gnf_s[...], BF16))
    xim_s[4, sl, :] = jnp.zeros((rows, T), F32)


def _fft32(load, emit, sign):
    half = N1 // 2
    for par in range(2):
        xs = []
        for n in range(half):
            a, b = load(n), load(n + half)
            xs.append(_cadd(a, b) if par == 0 else _cmul_const(_csub(a, b), n, N1, sign))
        out = _fft(xs, sign)
        for q in range(half):
            emit(2 * q + par, out[q])


def _b_s_pass1(xre_s, xim_s, ys_s, c, j):
    off = pl.multiple_of(j * 8, 8)

    def load(n1):
        rows = pl.ds(N2 * n1 + off, 8)
        return xre_s[c, rows, :], xim_s[c, rows, :]

    def emit(k1, v):
        ys_s[k1, c, pl.ds(pl.multiple_of(j * 16, 16), 16), :] = jnp.concatenate(v, axis=0).astype(BF16)
    _fft32(load, emit, -1)


def _b_s_pass2_fwd(ys_s, gsf_s, k1):
    rhs = jnp.concatenate([ys_s[k1, c] for c in range(NCT)], axis=1)
    return _dot(_ld(gsf_s, k1), rhs)


def _b_s_pass2_inv(vv, zs_s, wt_s, gsi_s, k1):
    outs = []
    for c in range(NCT):
        wd = wt_s[c, pl.ds(k1, N2, stride=N1), :]
        wr = pltpu.bitcast(wd << 16, F32)
        wi = pltpu.bitcast(wd & jnp.uint32(0xFFFF0000), F32)
        pcs = []
        for j in range(8):
            vr = vv[16 * j:16 * j + 8, c * T:(c + 1) * T]
            vi = vv[16 * j + 8:16 * j + 16, c * T:(c + 1) * T]
            a, b = wr[8 * j:8 * j + 8], wi[8 * j:8 * j + 8]
            pcs.append(vr * a - vi * b)
            pcs.append(vr * b + vi * a)
        outs.append(jnp.concatenate(pcs, axis=0).astype(BF16))
    ginv = _ld(gsi_s, k1)
    for c in range(NCT):
        zs_s[k1, c] = _dot(ginv, outs[c]).astype(BF16)


def _b_s_pass2(ys_s, zs_s, wt_s, gsf_s, gsi_s, k1s):
    pend = []
    for a in range(len(k1s) + P2D):
        if a < len(k1s):
            pend.append(_b_s_pass2_fwd(ys_s, gsf_s, k1s[a]))
        if a >= P2D:
            _b_s_pass2_inv(pend.pop(0), zs_s, wt_s, gsi_s, k1s[a - P2D])


def _b_s_pass3(zs_s, xre_s, xim_s, c, j, chain):
    off = pl.multiple_of(j * 8, 8)

    def load(k1):
        z = zs_s[k1, c, pl.ds(pl.multiple_of(j * 16, 16), 16), :].astype(F32)
        return z[0:8], z[8:16]

    def emit(n1, v):
        rows = pl.ds(N2 * n1 + off, 8)
        xre_s[c, rows, :] = v[0]
        xim_s[c, rows, :] = v[1]
        if chain and n1 >= N1 - 2:
            zs_s[N1, 0, 0:16, :] = jnp.concatenate(v, axis=0).astype(BF16)
    _fft32(load, emit, +1)


def _b_d_inverse(xre_s, xim_s, gdi_s, gni_s, yb_s, r0, rows):
    sl = pl.ds(r0, rows)
    us = []
    for p in range(4):
        lhs = jnp.concatenate([xre_s[p, sl, :], xim_s[p, sl, :]], axis=1).astype(BF16)
        o = _dot(lhs, _ld(gdi_s, p))
        us.append((o[:, :T], o[:, T:]))
    u0 = us[0][0] + _dot(xre_s[4, sl, :].astype(BF16), pltpu.bitcast(gni_s[...], BF16))
    u4 = us[0][1]
    (u1r, u1i), (u2r, u2i), (u3r, u3i) = us[1], us[2], us[3]
    e0, e1 = u0 + u4, u0 - u4
    ev = (e0 + u2r, e1 - u2i, e0 - u2r, e1 + u2i)
    pq, qq = u1r - u3r, u1i + u3i
    k = math.sqrt(0.5)
    od = (u1r + u3r, (pq - qq) * k, u3i - u1i, (pq + qq) * (-k))
    for a in range(4):
        yb_s[sl, a * T:(a + 1) * T] = (ev[a] + od[a]).astype(BF16)
        yb_s[sl, (a + 4) * T:(a + 5) * T] = (ev[a] - od[a]).astype(BF16)


VSL = 16
BQ = 128
ADEPTH = 2
ACK = 128
AORD = 3
AUN = 2


def _attn_order(h0):
    n = S // BQ
    if AORD == 0:
        return [(h0 + u, i) for u in range(AUN) for i in range(n - 1, -1, -1)]
    if AORD == 1:
        return [p for i in range(n) for p in ((h0, n - 1 - i), (h0 + 1, i))]
    if AORD >= 2:
        o = []
        lo, hi = 0, n - 1
        while lo <= hi:
            o.append(hi)
            hi -= 1
            if lo <= hi:
                o.append(lo)
                lo += 1
        if AORD == 2:
            return [(h0 + u, i) for u in range(AUN) for i in o]
        if AORD == 3:
            return [(h0 + u, i) for i in o for u in range(AUN)]
        if AORD == 4:
            return [(h0, i) for i in o] + [(h0 + 1, i) for i in o[::-1]]
        if AORD == 5:
            return [p for a, b in zip(o, o[::-1]) for p in ((h0, a), (h0 + 1, b))]


def _attn_heads(q_s, k_s, v_s, o_s, h0, ho):
    nt = BQ // T
    row = lax.broadcasted_iota(jnp.int32, (T, T), 0)
    col = lax.broadcasted_iota(jnp.int32, (T, T), 1)
    causal = col <= row

    def scores(h, i):
        r0 = i * BQ
        nfull = r0 // T + 1
        tiles = {}
        s = _dot_nt(_ld(q_s, h, _rows(r0, BQ)), _ld(k_s, h, _rows(0, nfull * T)))
        for t in range(nt):
            for j in range(nfull):
                tiles[t, j] = s[t * T:(t + 1) * T, j * T:(j + 1) * T]
        for t in range(1, nt):
            j = nfull - 1 + t
            st = _dot_nt(_ld(q_s, h, _rows(r0 + t * T, BQ - t * T)), _ld(k_s, h, _rows(j * T, T)))
            for u in range(t, nt):
                tiles[u, j] = st[(u - t) * T:(u - t + 1) * T]
        for t in range(nt):
            jd = nfull - 1 + t
            tiles[t, jd] = jnp.where(causal, tiles[t, jd], MASK_VAL)
        return tiles

    mlow = [None]

    def softmax_pv(h, i, tiles):
        r0 = i * BQ
        nfull = r0 // T + 1
        for t in range(nt):
            nk = nfull + t
            mx = tiles[t, 0]
            for j in range(1, nk):
                mx = jnp.maximum(mx, tiles[t, j])
            m = jnp.max(mx, axis=1, keepdims=True)
            if nk < S // T:
                mlow[0] = m if mlow[0] is None else jnp.minimum(mlow[0], m)
            lacc = o = None
            cj = ACK // T
            for j0 in range(0, nk, cj):
                ps = []
                for j in range(j0, min(nk, j0 + cj)):
                    p = jnp.exp2(tiles[t, j] - m)
                    lacc = p if lacc is None else lacc + p
                    ps.append(p)
                pc = jnp.concatenate(ps, axis=1) if len(ps) > 1 else ps[0]
                oo = _dot(pc.astype(BF16), _ld(v_s, h, _rows(j0 * T, len(ps) * T)))
                o = oo if o is None else o + oo
            l = jnp.sum(lacc, axis=1, keepdims=True)
            o_s[h - h0 + ho, _rows(r0 + t * T, T)] = _pk(o * pl.reciprocal(l, approx=True))

    hs = [h0 + u for u in range(AUN)]
    order = [(hs[u], i) for u, i in _attn_order(0)]
    pend = []
    for a in range(len(order) + ADEPTH):
        if a < len(order):
            pend.append(scores(*order[a]))
        if a >= ADEPTH:
            softmax_pv(*order[a - ADEPTH], pend.pop(0))

    @pl.when(jnp.min(mlow[0]) < MASK_VAL + 200.0)
    def _():
        def redo(n, c):
            u, t = n // (S // T), n % (S // T)
            h = h0 + u
            rows = pl.ds(pl.multiple_of(t * (T // 2), T // 2), T // 2)
            sf = _dot_nt(_ld(q_s, h, rows), _ld(k_s, h, _rows(0, S)))
            ri = lax.broadcasted_iota(jnp.int32, (T, S), 0) + t * T
            ci = lax.broadcasted_iota(jnp.int32, (T, S), 1)
            sf = jnp.where(ci <= ri, sf, MASK_VAL)
            pf = jnp.exp2(sf - jnp.max(sf, axis=1, keepdims=True))
            lf = jnp.sum(pf, axis=1, keepdims=True)
            of = _dot(pf.astype(BF16), _ld(v_s, h, _rows(0, S)))
            o_s[ho + u, rows] = _pk(of * pl.reciprocal(lf, approx=True))
            return c
        lax.fori_loop(0, AUN * (S // T), redo, 0)


HS = S // 2


def _lhs_sums(a11, a12, a21, a22):
    return (a11 + a22, a21 + a22, a11 + a12, a21 - a11, a12 - a22)


def _rhs_ops(b11, b12, b21, b22):
    return (b11 + b22, b11, b12 - b22, b21 - b11, b22, b11 + b12, b21 + b22)


def _strassen(lhs, rhs):
    m3, m4 = _dot(lhs[2], rhs[2]), _dot(lhs[3], rhs[3])
    m1, m2, m5, m6, m7 = [_dot(lhs[j], rhs[j]) for j in (0, 1, 4, 5, 6)]
    return (((m1 + m4) - m5) + m7, m3 + m5, m2 + m4, ((m1 - m2) + m3) + m6)


PR = 256
OR = 128
BR = 512
DSUB = 64
P2D = 1
P2U = 8
WSL = 16
WSL2 = 32
OCH = 1
AREP = 1
DMA_A = 4
DMA_B = 32
DSUB2 = 128
WPIN = 0
PORD = 3
WORD = 3
NWO = 16


def _kernel(ax_hbm, ac_hbm, wq_hbm, wuk_hbm, wuv_hbm, wo_hbm, bx_hbm, wrT_hbm, wiT_hbm,
            gdf_hbm, gnf_hbm, gdi_hbm, gni_hbm, gsf_hbm, gsi_hbm,
            out_hbm,
            ax_s, ac_s, w_st, wo_s, zs_s, gdi_s, gni_s, sems, wosem):
    def copy(src, dst, i):
        return pltpu.make_async_copy(src, dst, sems.at[i])

    def wcopies(g):
        hs = pl.ds(pl.multiple_of(g * 8, 8), 8)
        return (copy(wq_hbm.at[:, hs, :], w_st.at[pl.ds(0, DM)], 2),
                copy(wuk_hbm.at[:, hs, :], w_st.at[pl.ds(DM, DC)], 3),
                copy(wuv_hbm.at[:, hs, :], w_st.at[pl.ds(DM + DC, DC)], 4))

    def wocopies(u):
        r = pl.multiple_of(u * T, T)
        r2 = pl.multiple_of(H * HD // 2 + u * T, T)
        return (pltpu.make_async_copy(wo_hbm.at[pl.ds(r, T), :], wo_s.at[pl.ds(r, T), :], wosem.at[2 * u]),
                pltpu.make_async_copy(wo_hbm.at[pl.ds(r2, T), :], wo_s.at[pl.ds(r2, T), :], wosem.at[2 * u + 1]))

    def b_phase(bx_s, y_s, wrT_s, wiT_s, wd_s, wt_s, xre_s, xim_s, ys_s,
                gdf_s, gnf_s, gsf_s, gsi_s, bsem):
        def bcopy(src, dst, i):
            return pltpu.make_async_copy(src, dst, bsem.at[i])
        nch = S // BR
        xc = [bcopy(bx_hbm.at[pl.ds(i * BR, BR), :], bx_s.at[pl.ds(i * BR, BR), :], i)
              for i in range(nch)]
        cc = [bcopy(gdf_hbm, gdf_s, nch), bcopy(gnf_hbm, gnf_s, nch + 1),
              bcopy(wrT_hbm, wrT_s, nch + 2), bcopy(wiT_hbm, wiT_s, nch + 3),
              bcopy(gsf_hbm, gsf_s, nch + 4), bcopy(gsi_hbm, gsi_s, nch + 5)]
        xc[0].start()
        cc[0].start()
        cc[1].start()
        xc[1].start()

        cc[0].wait()
        cc[1].wait()
        xc[0].wait()
        xc[2].start()
        _b_d_forward_vpu(bx_s, y_s, 0, 0, BR)

        for i in range(nch):
            if i + 1 < nch:
                xc[i + 1].wait()
            if i == 0:
                xc[3].start()
            if i == 2:
                cc[2].start()
                cc[3].start()
            for a in range(0, BR, DSUB):
                _b_d_forward_mxu(y_s, i % 2, gdf_s, gnf_s, xre_s, xim_s, i * BR, a, DSUB)
                if i + 1 < nch:
                    for b in range(a, a + DSUB, VSL):
                        _b_d_forward_vpu_slab(bx_s, y_s, (i + 1) % 2, (i + 1) * BR, b)

        cc[2].wait()
        cc[3].wait()
        cc[4].start()
        cc[5].start()
        copy(ac_hbm, ac_s, 1).start()

        def p1(i, c):
            @pl.when(i == DMA_A)
            def _():
                copy(ax_hbm, ax_s, 0).start()
            for v in range(2):
                _b_prepare_w_order(wrT_s, wiT_s, wd_s, wt_s, 2 * i + v)
            for v in range(NCT):
                u = i * NCT + v
                _b_s_pass1(xre_s, xim_s, ys_s, u // 8, u % 8)
            for v in range(2):
                _b_prepare_w_words(wrT_s, wiT_s, wd_s, jnp.minimum(2 * i + 2 + v, S // T - 1))
            return c
        for v in range(2):
            _b_prepare_w_words(wrT_s, wiT_s, wd_s, v)
        lax.fori_loop(0, 8, p1, 0)
        cc[4].wait()
        cc[5].wait()
        copy(ac_hbm, ac_s, 1).wait()
        for cp in wcopies(0):
            cp.start()

        npi = N1 // P2U

        def p2(kk, c):
            @pl.when(kk == npi - 1)
            def _():
                for v in range(NWO):
                    for cp in wocopies(v):
                        cp.start()
                copy(gdi_hbm, gdi_s, 8).start()
                copy(gni_hbm, gni_s, 9).start()
            _b_s_pass2(ys_s, zs_s, wt_s, gsf_s, gsi_s, [kk * P2U + u for u in range(P2U)])
            return c
        lax.fori_loop(0, N1 // P2U, p2, 0)

    def b_scope():
      pl.run_scoped(
        b_phase,
        pltpu.VMEM((S, DM), BF16), pltpu.VMEM((2, BR // 2, DM), U32),
        pltpu.VMEM((DF, S), BF16), pltpu.VMEM((DF, S), BF16),
        pltpu.VMEM((S // T, 512, T), U32), pltpu.VMEM((NCT, S, T), U32),
        pltpu.VMEM((NCT, S, T), F32), pltpu.VMEM((NCT, S, T), F32),
        pltpu.VMEM((N1, NCT, T, T), BF16),
        pltpu.VMEM((4, 128, 256), U32), pltpu.VMEM((T // 2, T), U32),
        pltpu.VMEM((N1, T // 2, T), U32), pltpu.VMEM((N1, T // 2, T), U32),
        pltpu.SemaphoreType.DMA((S // BR + 6,)),
    )

    def a_outer(ctx_s, wos_s):
        def a_main(wu_s, q_s, k_s, v_s):
            def stage_w(i, chain):
                rows = (DM + 2 * DC) // 8
                step = WSL2 if chain else 128
                for a in range(0, rows, step):
                    r = pl.multiple_of(i * rows + a, step)
                    v = w_st[pl.ds(r, step)]
                    wu_s[pl.ds(pl.multiple_of(4 * r, 4 * step), 4 * step), :] = pltpu.bitcast(
                        v.reshape(step * 8, HD), U32)
                    if chain:
                        w_st[DM + 2 * DC:DM + 2 * DC + 2] = v[0:2]

            def w_rhs(slot, base, kk):
                def blk(m0, hp0):
                    cols = []
                    for hp in (hp0, hp0 + 1):
                        x = wu_s[pl.ds(4 * m0 + hp, kk, stride=4), :]
                        cols.append(pltpu.bitcast(x << 16, F32))
                        cols.append(pltpu.bitcast(x & jnp.uint32(0xFFFF0000), F32))
                    return jnp.concatenate(cols, axis=1)
                b11, b12 = blk(base, 0), blk(base, 2)
                b21, b22 = blk(base + kk, 0), blk(base + kk, 2)
                return [v.astype(BF16) for v in _rhs_ops(b11, b12, b21, b22)]

            def prep_wo(u, chain):
                step = WSL if chain else T
                for a in range(0, T, step):
                    r = pl.multiple_of(u * T + a, step)
                    top = wo_s[pl.ds(r, step), :].astype(F32)
                    bot = wo_s[pl.ds(H * HD // 2 + r, step), :].astype(F32)
                    ops = _rhs_ops(top[:, :512], top[:, 512:], bot[:, :512], bot[:, 512:])
                    r2 = pl.multiple_of(u * (T // 2) + a // 2, step // 2)
                    for j in range(7):
                        v = ops[j].astype(BF16)
                        wos_s[j, pl.ds(r2, step // 2), :] = pltpu.bitcast(v, U32)
                    if chain:
                        wo_s[H * HD:H * HD + 16, 0:HD] = v[0:16, 0:HD]

            copy(ax_hbm, ax_s, 0).wait()
            for cp in wcopies(0):
                cp.wait()

            def prew(i, c):
                stage_w(i, False)
                return c
            lax.fori_loop(0, 8, prew, 0)

            def lhs7(src, r):
                kk = src.shape[1] // 2
                top, bot = pl.ds(r, PR), pl.ds(HS + r, PR)
                a11, a12, a21, a22 = src[top, :kk], src[top, kk:], src[bot, :kk], src[bot, kk:]
                sm = [v.astype(BF16) for v in _lhs_sums(*[v.astype(F32) for v in (a11, a12, a21, a22)])]
                return (sm[0], sm[1], a11, a22, sm[2], sm[3], sm[4])

            def group(g, c):
                slot = 0
                gn = jnp.minimum(g + 1, NG - 1)
                for cp in wcopies(gn):
                    cp.start()

                def chunk(i, cc):
                    r = pl.multiple_of(i * PR, PR)
                    top, bot = pl.ds(r, PR), pl.ds(HS + r, PR)
                    for cp in wocopies(g * 4 + i):
                        cp.wait()

                    def put(dst, cs, scale=None):
                        top2 = pl.ds(pl.multiple_of(i * (PR // 2), PR // 2), PR // 2)
                        bot2 = pl.ds(pl.multiple_of(HS // 2 + i * (PR // 2), PR // 2), PR // 2)
                        for cb, rows, h0 in zip(cs, (top2, top2, bot2, bot2), (0, 4, 0, 4)):
                            if scale is not None:
                                cb = cb * scale
                            cb = _pk(cb)
                            for hh in range(4):
                                dst[h0 + hh, rows, :] = cb[:, hh * HD:(hh + 1) * HD]
                    cl = lhs7(ac_s, r)
                    kcs = _strassen(cl, w_rhs(slot, DM, DC // 2))
                    put(k_s, kcs)
                    if WPIN == 1:
                        wo_s[H * HD:H * HD + 16, 0:HD] = kcs[1][0:16, 0:HD].astype(BF16)
                        prep_wo(g * 4 + i, True)
                    put(v_s, _strassen(cl, w_rhs(slot, DM + DC, DC // 2)))
                    put(q_s, _strassen(lhs7(ax_s, r), w_rhs(slot, 0, DM // 2)), Q_SCALE)
                    if WPIN == 0: prep_wo(g * 4 + i, True)
                    return cc
                lax.fori_loop(0, HS // PR, chunk, 0)

                for cp in wcopies(gn):
                    cp.wait()

                def head(hh, cc):
                    h = hh * AUN
                    _attn_heads(q_s, k_s, v_s, ctx_s, h, g * 8 + h)
                    for u in range(AUN):
                        stage_w(h + u, True)
                    return cc
                lax.fori_loop(0, 8 // AUN, head, 0)
                return c
            lax.fori_loop(0, NG, group, 0)

        b_scope()
        pl.run_scoped(a_main, pltpu.VMEM((4 * (DM + 2 * DC), HD), U32),
                      *[pltpu.VMEM((8, S // 2, HD), U32)] * 3)

        def a_out(oa_s, yb_s, xre_s, xim_s, osem):
            nch = HS // OR

            def ocopies(i):
                r = pl.multiple_of(i * OR, OR)
                r2 = pl.multiple_of(HS + i * OR, OR)
                return (pltpu.make_async_copy(oa_s.at[pl.ds(r, OR), :],
                                              out_hbm.at[pl.ds(r, OR), pl.ds(0, DM)], osem.at[2 * i]),
                        pltpu.make_async_copy(oa_s.at[pl.ds(r2, OR), :],
                                              out_hbm.at[pl.ds(r2, OR), pl.ds(0, DM)], osem.at[2 * i + 1]))

            def ycopy(i):
                r = pl.multiple_of(i * DSUB2, DSUB2)
                return pltpu.make_async_copy(yb_s.at[pl.ds(r, DSUB2), :],
                                             out_hbm.at[pl.ds(r, DSUB2), pl.ds(DM, DM)], osem.at[16 + i])

            def blk(rows, h0):
                return [_ld(ctx_s, h0 + h, rows) for h in range(H // 2)]

            def ochunk(i, c):
                r = pl.multiple_of(i * OR, OR)
                top, bot = pl.ds(r, OR), pl.ds(HS + r, OR)
                cat = lambda xs: jnp.concatenate(xs, axis=1)
                hk = H * HD // 2
                top2 = pl.ds(pl.multiple_of(i * (OR // 2), OR // 2), OR // 2)
                bot2 = pl.ds(pl.multiple_of(HS // 2 + i * (OR // 2), OR // 2), OR // 2)
                a11, a22 = cat(blk(top2, 0)), cat(blk(bot2, 16))
                m3 = _dot(a11, _ld(wos_s, 2))
                m4 = _dot(a22, _ld(wos_s, 3))
                a12, a21 = cat(blk(top2, 16)), cat(blk(bot2, 0))
                sums = [v.astype(BF16) for v in
                        _lhs_sums(*[v.astype(F32) for v in (a11, a12, a21, a22)])]
                m1 = _dot(sums[0], _ld(wos_s, 0))
                m2 = _dot(sums[1], _ld(wos_s, 1))
                m5 = _dot(sums[2], _ld(wos_s, 4))
                m6 = _dot(sums[3], _ld(wos_s, 5))
                m7 = _dot(sums[4], _ld(wos_s, 6))
                cs = (((m1 + m4) - m5) + m7, m3 + m5, m2 + m4, ((m1 - m2) + m3) + m6)
                for cb, rows, c0 in zip(cs, (top, top, bot, bot), (0, 512, 0, 512)):
                    oa_s[rows, c0:c0 + 512] = cb.astype(BF16)
                for v in range(NCT * 8 // nch):
                    u = i * (NCT * 8 // nch) + v
                    _b_s_pass3(zs_s, xre_s, xim_s, u // 8, u % 8, True)
                for cp in ocopies(i):
                    cp.start()
                return c
            lax.fori_loop(0, nch, ochunk, 0)

            copy(gdi_hbm, gdi_s, 8).wait()
            copy(gni_hbm, gni_s, 9).wait()

            def dinv(i, c):
                for a in range(BR // DSUB2):
                    r = pl.multiple_of(i * BR + a * DSUB2, DSUB2)
                    _b_d_inverse(xre_s, xim_s, gdi_s, gni_s, yb_s, r, DSUB2)
                for a in range(BR // DSUB2):
                    ycopy(i * (BR // DSUB2) + a).start()
                return c
            lax.fori_loop(0, S // BR, dinv, 0)
            for i in range(nch):
                for cp in ocopies(i):
                    cp.wait()
            for i in range(S // DSUB2):
                ycopy(i).wait()

        pl.run_scoped(a_out, pltpu.VMEM((S, DM), BF16), pltpu.VMEM((S, DM), BF16),
                      pltpu.VMEM((NCT, S, T), F32), pltpu.VMEM((NCT, S, T), F32),
                      pltpu.SemaphoreType.DMA((16 + S // DSUB2,)))

    pl.run_scoped(a_outer, pltpu.VMEM((H, S // 2, HD), U32), pltpu.VMEM((7, H * HD // 4, 512), U32))


@jax.jit
def pallas_concat_heads__compressed_kv_cla__spectral_gfnet__prompt_kernel(
    A_x, A_c_kv, A_w_q, A_w_uk, A_w_uv, A_w_o, B_x, B_w_r, B_w_i,
):
    hbm = pl.BlockSpec(memory_space=pl.ANY)
    out = pl.pallas_call(
        _kernel,
        in_specs=[hbm] * 15,
        out_specs=hbm,
        out_shape=jax.ShapeDtypeStruct((S, 2 * DM), BF16),
        scratch_shapes=[
            pltpu.VMEM((S, DM), BF16), pltpu.VMEM((S, DC), BF16),
            pltpu.VMEM((DM + 2 * DC + 2, 8, HD), BF16),
            pltpu.VMEM((H * HD + 16, DM), BF16),
            pltpu.VMEM((N1 + 1, NCT, T, T), BF16),
            pltpu.VMEM((4, 128, 256), U32), pltpu.VMEM((T // 2, T), U32),
            pltpu.SemaphoreType.DMA((10,)), pltpu.SemaphoreType.DMA((2 * NWO,)),
        ],
        compiler_params=pltpu.CompilerParams(vmem_limit_bytes=120 * 1024 * 1024),
    )(A_x.reshape(S, DM), A_c_kv.reshape(S, DC), A_w_q, A_w_uk, A_w_uv,
      A_w_o.reshape(H * HD, DM), B_x.reshape(S, DM), B_w_r.T, B_w_i.T, *_CONSTS)
    return out.reshape(1, S, 2 * DM)
```
